```python
import jax
import jax.numpy as jnp

def _softmax(x, axis=-1):
    return jax.nn.softmax(x, axis=axis)
def _gelu(x):
    return jax.nn.gelu(x, approximate=True)
def _silu(x):
    return jax.nn.silu(x)
def _sigmoid(x):
    return jax.nn.sigmoid(x)
def _layernorm(x, axis=-1, eps=1e-5):
    m = jnp.mean(x, axis=axis, keepdims=True)
    v = jnp.var(x, axis=axis, keepdims=True)
    return (x - m) / jnp.sqrt(v + eps)
def _scatter_add(tgt, idx, src, axis=0):
    return tgt.at[idx].add(src)
def _segment_sum(src, seg, n):
    return jax.ops.segment_sum(src, seg, n)
class _Rng:
    def __init__(self, key):
        self._k = key
    def _next(self):
        self._k, sub = jax.random.split(self._k)
        return sub
    def normal(self, shape):
        return jax.random.normal(self._next(), shape, dtype=jnp.bfloat16)
    def randint(self, lo, hi, shape):
        return jax.random.randint(self._next(), shape, lo, hi, dtype=jnp.int32)
    def uniform(self, shape, lo=0.0, hi=1.0):
        return jax.random.uniform(self._next(), shape, jnp.bfloat16, lo, hi)
    def permutation(self, n):
        return jax.random.permutation(self._next(), n)


kernel_name = 'recurrent_scan__linear_kernel_hedgehog__moe_arch_mod__prompt'

def setup_inputs():
    _rng = _Rng(jax.random.key(int.from_bytes(__import__("os").urandom(4), "little")))
    _w = (lambda a: (lambda t: t.astype(jnp.bfloat16) if jnp.issubdtype(t.dtype, jnp.floating) else t)(jnp.asarray(a)))
    def _A_setup():
        B, S, D, H = 1, 2048, 1024, 32
        Dh = D // H
        return {
            "x": _w((lambda *s: _rng.normal(s) * 0.05)(B, S, D)),
            "wqkv": _w((lambda *s: _rng.normal(s) * 0.05)(D, 3 * D)),
            "w_phi": _w((lambda *s: _rng.normal(s) * 0.05)(H, Dh, Dh) * (Dh ** -0.5)),
            "wo": _w((lambda *s: _rng.normal(s) * 0.05)(D, D)),
        }
    _A_in = _A_setup()

    def _B_setup():
        B, S, D, F, C = 1, 2048, 1024, 3584, 1
        return {
            "x": _w((lambda *s: _rng.normal(s) * 0.05)(B, S, D)),
            "w_r": _w((lambda *s: _rng.normal(s) * 0.05)(D)),
            "w_gate": _w((lambda *s: _rng.normal(s) * 0.05)(D, F)),
            "w_up": _w((lambda *s: _rng.normal(s) * 0.05)(D, F)),
            "w_down": _w((lambda *s: _rng.normal(s) * 0.05)(F, D)),
        }
    _B_in = _B_setup()

    return {
        "A_x": _A_in["x"],
        "A_wqkv": _A_in["wqkv"],
        "A_w_phi": _A_in["w_phi"],
        "A_wo": _A_in["wo"],
        "B_x": _B_in["x"],
        "B_w_r": _B_in["w_r"],
        "B_w_gate": _B_in["w_gate"],
        "B_w_up": _B_in["w_up"],
        "B_w_down": _B_in["w_down"],
    }

def reference(A_x, A_wqkv, A_w_phi, A_wo, B_x, B_w_r, B_w_gate, B_w_up, B_w_down):
    def _A_ref(x, wqkv, w_phi, wo):
        B, S, D = x.shape
        H = 32; Dh = D // H
        qkv = (lambda x, *d: x.transpose(*d))((x @ wqkv).reshape(B, S, 3, H, Dh), 2, 0, 3, 1, 4)
        q, k, v = qkv[0], qkv[1], qkv[2]
        pq = jnp.einsum("bhsd,hdf->bhsf", q, w_phi)
        pk = jnp.einsum("bhsd,hdf->bhsf", k, w_phi)
        phi_q = jnp.concatenate([_softmax(pq, axis=-1), _softmax(-pq, axis=-1)], axis=-1)
        phi_k = jnp.concatenate([_softmax(pk, axis=-1), _softmax(-pk, axis=-1)], axis=-1)
        kv = jnp.einsum("bhsf,bhsd->bhfd", phi_k, v)
        z  = jnp.einsum("bhsf->bhf", phi_k)
        num = jnp.einsum("bhqf,bhfd->bhqd", phi_q, kv)
        den = jnp.einsum("bhqf,bhf->bhq", phi_q, z)[..., None] + 1e-6
        o = num / den
        return (lambda x, *d: x.transpose(*d))(o, 0, 2, 1, 3).reshape(B, S, D) @ wo

    def _B_ref(x, w_r, w_gate, w_up, w_down):
        B, S, D = x.shape
        C = 1
        r = x @ w_r
        idx = jnp.argsort(-r, axis=-1)[:, :C]
        idx_e = jnp.repeat(idx.reshape(B, C, 1), D, axis=2)
        x_sel = jnp.take_along_axis(x, idx_e, axis=1)
        g = _silu(x_sel @ w_gate)
        u = x_sel @ w_up
        y = (g * u) @ w_down
        r_sel = _sigmoid(jnp.take_along_axis(r, idx, axis=1))
        y = y * r_sel.reshape(B, C, 1)
        b_off = (jnp.arange(B) * S).reshape(B, 1)
        flat_idx = (idx + b_off).reshape(B * C)
        zero = (x * 0.0).reshape(B * S, D)
        upd = _scatter_add(zero, flat_idx, y.reshape(B * C, D), axis=0)
        return x + upd.reshape(B, S, D)

    x = A_x
    xn = _layernorm(x, axis=-1)
    s = _A_ref(xn, A_wqkv, A_w_phi, A_wo)
    g = _silu(_B_ref(xn, B_w_r, B_w_gate, B_w_up, B_w_down))
    return x + s * g
```

```python
import math

import jax
import jax.numpy as jnp
from jax import lax
import jax.experimental.pallas as pl
import jax.experimental.pallas.tpu as pltpu

S, D, H, DH, F = 2048, 1024, 32, 32, 3584
SUB = 128
STEP = 2 * SUB
NSTEP = S // STEP
NB = 4
FC = F // NB
HD = D // 2
NG = HD // 128
FLUSH_AT = [(3, 6), (6,), (5,), (4, 6)][0]
X_CUTS = (0, 1, 2, 5, 8)
NPAIR = H // 2
LOG2E = math.log2(math.e)
EPS = 1.0013580322265625e-05
F32, BF16, U32 = jnp.float32, jnp.bfloat16, jnp.uint32

NT_DIMS = (((1,), (1,)), ((), ()))


def _dot(a, b):
    return jnp.dot(a, b, preferred_element_type=F32)


def _dot_nt(a, b):
    return lax.dot_general(a, b, NT_DIMS, preferred_element_type=F32)


def _round_bf16(v):
    return v.astype(BF16).astype(F32)


def _pack(v):
    return pltpu.bitcast(v.astype(BF16), U32)


def _unpack(v):
    return pltpu.bitcast(v, BF16)


def _silu(t):
    h = 0.5 * t
    return h + h * jnp.tanh(h)


def _recip(d):
    r = pltpu.reciprocal(d, approx=True)
    return r * (2.0 - d * r)


def _allreduce(v, op):
    v = op(v, pltpu.roll(v, 4, 0))
    return op(v, pltpu.roll(v, 2, 0))


def _tree(vals, op):
    vals = list(vals)
    while len(vals) > 1:
        nxt = [op(vals[i], vals[i + 1]) for i in range(0, len(vals) - 1, 2)]
        if len(vals) % 2:
            nxt.append(vals[-1])
        vals = nxt
    return vals[0]


def _dual_softmax(p):
    ps = [p[8 * j:8 * j + 8] for j in range(8)]
    mx = _allreduce(_tree(ps, jnp.maximum), jnp.maximum)
    mn = _allreduce(_tree(ps, jnp.minimum), jnp.minimum)
    ep = [jnp.exp2(v - mx) for v in ps]
    en = [jnp.exp2(mn - v) for v in ps]
    rp = _recip(_allreduce(_tree(ep, jnp.add), jnp.add))
    rn = _recip(_allreduce(_tree(en, jnp.add), jnp.add))
    return [e * rp for e in ep] + [e * rn for e in en]


def _lhs_sums(a11, a12, a21, a22):
    return (a11 + a22, a21 + a22, a11, a22, a11 + a12, a21 - a11, a12 - a22)


def _rhs_sums(b11, b12, b21, b22):
    return (b11 + b22, b11, b12 - b22, b21 - b11, b22, b11 + b12, b21 + b22)


def _strassen(prod, emit, between=None):
    between = between or (lambda n: None)
    m2 = prod(1)
    between(0)
    m4 = prod(3)
    emit(1, 0, m2 + m4)
    between(1)
    m3 = prod(2)
    c22 = m3 - m2
    between(2)
    m5 = prod(4)
    emit(0, 1, m3 + m5)
    c11 = m4 - m5
    between(3)
    m1 = prod(0)
    c11 = c11 + m1
    c22 = c22 + m1
    between(4)
    emit(0, 0, c11 + prod(6))
    between(5)
    emit(1, 1, c22 + prod(5))
    between(6)


class _Scope:
    def __init__(self, name):
        self.s = jax.named_scope(name) if 0 else None

    def __enter__(self):
        if self.s:
            self.s.__enter__()

    def __exit__(self, *a):
        if self.s:
            self.s.__exit__(*a)


def _kernel(x_hbm, wqkv_hbm, wphi_hbm, wo_hbm, wr_hbm, wg_hbm, wu_hbm, wd_hbm,
            out_hbm,
            x_buf, xs_buf, stat_buf, w_raw, w_sum, wo_sum, wphi_buf, bd_buf, wr_buf,
            pq_buf, vt_buf, phik_buf, kv_acc, z_acc, kvb_buf, os_buf,
            wg_buf, wu_buf, wd_buf, xb_buf, y_acc, upd_buf, out_buf,
            sem_x, sem_q, sem_w, sem_s, sem_f, sem_o, sem_last, sem_order):
    def x_copy(n):
        rows = pl.ds(X_CUTS[n] * STEP, (X_CUTS[n + 1] - X_CUTS[n]) * STEP)
        return pltpu.make_async_copy(x_hbm.at[rows], x_buf.at[rows], sem_x.at[n])

    def q_copy(g):
        cols = pl.ds(128 * g, 128)
        return pltpu.make_async_copy(wqkv_hbm.at[:, cols], w_raw.at[0, :, cols], sem_q.at[g])

    def w_copy(m):
        return pltpu.make_async_copy(wqkv_hbm.at[:, pl.ds(m * D, D)], w_raw.at[m], sem_w.at[m - 1])

    def f_copies(i):
        return (
            pltpu.make_async_copy(wg_hbm.at[:, pl.ds(i * FC, FC)], wg_buf.at[i], sem_f.at[i]),
            pltpu.make_async_copy(wu_hbm.at[:, pl.ds(i * FC, FC)], wu_buf.at[i], sem_f.at[NB + i]),
            pltpu.make_async_copy(wd_hbm.at[pl.ds(i * FC, FC)], wd_buf.at[i], sem_f.at[2 * NB + i]),
        ) + tuple(
            pltpu.make_async_copy(wo_hbm.at[:, cols], w_raw.at[3, :, cols], sem_f.at[(3 + half) * NB + i])
            for half in range(2)
            for cols in [pl.ds(pl.multiple_of(128 * (i + NG * half), 128), 128)])

    def o_copy(j):
        return pltpu.make_async_copy(
            out_buf.at[pl.ds(j * STEP, STEP)], out_hbm.at[pl.ds(j * STEP, STEP)], sem_o.at[j])

    wphi_copy = pltpu.make_async_copy(wphi_hbm, wphi_buf, sem_s.at[0])
    wr_copy = pltpu.make_async_copy(wr_hbm, wr_buf, sem_s.at[1])

    def fold_matrix(g):
        r = lax.broadcasted_iota(jnp.int32, (128, DH), 0)
        f = lax.broadcasted_iota(jnp.int32, (128, DH), 1)
        sel = jnp.where((r % 64) // 2 == f, 1.0, 0.0).astype(BF16)
        t = _dot_nt(sel, wphi_buf[pl.ds(128 * g, 128), :])
        r = lax.broadcasted_iota(jnp.int32, (128, 128), 0)
        c = lax.broadcasted_iota(jnp.int32, (128, 128), 1)
        return jnp.where(2 * (r // 64) + r % 2 == c // DH, t, 0.0)

    def prepare_weights(m, g):
        def block(half, k0):
            w = w_raw[m, pl.ds(k0, 256), pl.ds(pl.multiple_of(128 * (g + NG * half), 128), 128)]
            if m < 2:
                return _dot_nt(_unpack(bd_buf[g, :, pl.ds(128 * half, 128)]), w) * LOG2E
            return w.T.astype(F32)

        blocks = {k0: (block(0, k0), block(0, HD + k0), block(1, k0), block(1, HD + k0))
                  for k0 in range(0, HD, 256)}

        def store():
            dst = wo_sum if m == 3 else w_sum.at[m]
            for k0, quad in blocks.items():
                for n, v in enumerate(_lhs_sums(*quad)):
                    dst.at[n][pl.ds(pl.multiple_of(64 * g, 64), 64), pl.ds(k0, 256)] = _pack(v)
        return store

    best = [jnp.full((8, 128), -jnp.inf, F32), jnp.zeros((8, 128), F32)]

    def token_stats(j, never16):
        last = None
        wr = wr_buf[...].astype(F32)
        wrow = jnp.concatenate(
            [jnp.broadcast_to(wr[c:c + 1], (16, 128)) for c in range(8)], axis=1)
        sub = lax.broadcasted_iota(jnp.int32, (8, 128), 0).astype(F32)
        for r in range(0, STEP, 16):
            rows = pl.ds(j * STEP + r, 16)
            x = x_buf[rows, :].astype(F32)
            if last is not None:
                x = jnp.concatenate([jnp.where(never16, last, x[:, :128]), x[:, 128:]], axis=1)
            mean = jnp.sum(x, axis=1, keepdims=True) * (1.0 / D)
            c = x - mean
            var = jnp.sum(c * c, axis=1, keepdims=True) * (1.0 / D)
            inv = 1.0 / _round_bf16(jnp.sqrt(_round_bf16(_round_bf16(var) + EPS)))
            score = _round_bf16(jnp.sum(c * wrow, axis=1, keepdims=True) * inv)
            inv = jnp.broadcast_to(inv, (16, 128))
            stat_buf[0, rows, :] = jnp.broadcast_to(mean, (16, 128))
            stat_buf[1, rows, :] = inv
            if never16 is not None and (r // 16) % 2 == 0:
                last = inv
            score = jnp.broadcast_to(score, (16, 128))
            for hh in range(2):
                sc = score[8 * hh:8 * hh + 8]
                upd = sc > best[0]
                best[0] = jnp.where(upd, sc, best[0])
                best[1] = jnp.where(upd, sub + float(j * STEP + r + 8 * hh), best[1])
            yield

    def advance(gen, count):
        for _ in range(count):
            next(gen, None)

    def normalized(rows, cols=slice(None)):
        x = x_buf[rows, cols].astype(F32)
        reps = x.shape[1] // 128
        mean = jnp.concatenate([stat_buf[0, rows, :]] * reps, axis=1)
        inv = jnp.concatenate([stat_buf[1, rows, :]] * reps, axis=1)
        return x, (x - mean) * inv

    def token_sums(j):
        for r in range(0, SUB, 16):
            a = normalized(pl.ds(j * STEP + r, 16))[1]
            b = normalized(pl.ds(j * STEP + SUB + r, 16))[1]
            for n, v in enumerate(_rhs_sums(a[:, :HD], b[:, :HD], a[:, HD:], b[:, HD:])):
                xs_buf.at[j, n][pl.ds(r // 2, 8), :] = _pack(v)

    def project_in(m, j, emit, between=None):
        _strassen(lambda n: _dot_nt(_unpack(w_sum[m, n]), _unpack(xs_buf[j, n])), emit, between)

    def project_q(j, between=None, m=0):
        def emit(rh, ch, v):
            pq_buf[j, ch, pl.ds(rh * HD, HD), :] = v
        project_in(m, j, emit, between)

    class Deferred:
        def __init__(self):
            self.now = 0
            self.items = []

        def add(self, delay, fn):
            self.items.append((self.now + delay, fn))

        def tick(self):
            self.now += 1
            due = [fn for t, fn in self.items if t <= self.now]
            self.items = [(t, fn) for t, fn in self.items if t > self.now]
            for fn in due:
                fn()

        def flush(self):
            for _, fn in self.items:
                fn()
            self.items = []

    def start_in_order(copies):
        for c in copies:
            c.start(priority=1)
            pl.semaphore_signal(sem_order, 1)
            pl.semaphore_wait(sem_order, 1)

    start_in_order(
        [wr_copy, x_copy(0), wphi_copy]
        + [q_copy(g + NG * half) for g in range(NG) for half in range(2)]
        + [x_copy(1), x_copy(2), w_copy(2), w_copy(1), x_copy(3)]
        + [c for i in range(NB) for c in f_copies(i)])
    with _Scope("wr"):
        wr_copy.wait()
    with _Scope("wx0"):
        x_copy(0).wait()
    with _Scope("wphi"):
        wphi_copy.wait()
    advance(token_stats(0, None), STEP // 16)
    never = stat_buf[1, pl.ds(0, 8), :] < 0.0
    never16 = jnp.concatenate([never, never], axis=0)
    zero = never.astype(jnp.int32)[0, 0]
    token_sums(0)
    for g in range(NG):
        bd_buf.at[g][...] = _pack(jnp.concatenate([fold_matrix(g), fold_matrix(g + NG)], axis=1))
    for g in range(NG):
        with _Scope("wq%d" % g):
            q_copy(g).wait()
            q_copy(g + NG).wait()
        prepare_weights(0, g)()
    with _Scope("wx1"):
        x_copy(1).wait()
    per_product = [(4, 4, 4, 4, 0, 0, 0), (3, 3, 3, 3, 2, 2, 0), (3, 3, 2, 2, 2, 2, 2)][1]
    later = Deferred()
    for j in range(NSTEP - 1):
        if j == 1:
            with _Scope("wx2"):
                x_copy(2).wait()
        if j == 4:
            with _Scope("wkv"):
                w_copy(2).wait()
                w_copy(1).wait()
                x_copy(3).wait()
        stats = token_stats(j + 1, never16)

        def side(n, j=j, stats=stats):
            later.tick()
            advance(stats, per_product[n])
            t = 7 * (j - 4) + n
            if t >= 0 and t % 5 == 0 and t // 5 < NG:
                later.add(2, prepare_weights(1, t // 5))
            if t >= 0 and t % 5 == 2 and t // 5 < NG:
                later.add(2, prepare_weights(2, t // 5))
        project_q(j, side)
        token_sums(j + 1)
    later.flush()

    top = jnp.max(best[0], axis=0, keepdims=True)
    cand = jnp.where(best[0] == top, best[1], float(S))
    idx = jnp.min(cand, axis=0, keepdims=True).astype(jnp.int32)[0, 0]
    idx = jnp.clip(idx, 0, S - 1)
    slab = pl.ds(pl.multiple_of((idx // 16) * 16, 16), 16)
    pick = lax.broadcasted_iota(jnp.int32, (16, D), 0) == idx % 16
    x_sel = jnp.sum(jnp.where(pick, _round_bf16(normalized(slab)[1]), 0.0), axis=0, keepdims=True)
    for c in range(D // 128):
        xb_buf[pl.ds(128 * c, 128), :] = jnp.broadcast_to(
            x_sel[:, 128 * c:128 * c + 128], (128, 128)).T
    kv_acc[...] = jnp.zeros(kv_acc.shape, F32)
    z_acc[...] = jnp.zeros(z_acc.shape, F32)
    y_acc[...] = jnp.zeros(y_acc.shape, F32)

    def ffn(i):
        last = None
        ys = [y_acc[:, pl.ds(128 * n, 128)] for n in range(D // 128)]
        for c in range(FC // 128):
            res = []
            for w_buf in (wg_buf, wu_buf):
                acc = jnp.zeros((8, 128), F32)
                if last is not None:
                    acc = jnp.where(never, last, acc)
                for r in range(0, D, 8):
                    w = w_buf[i, pl.ds(r, 8), pl.ds(128 * c, 128)].astype(F32)
                    acc = acc + w * xb_buf[pl.ds(r, 8), :]
                last = acc
                res.append(_round_bf16(jnp.sum(acc, axis=0, keepdims=True)))
            h = _round_bf16(_round_bf16(_silu(res[0])) * res[1])
            hb = jnp.broadcast_to(h, (128, 128)).T
            for n in range(D // 128):
                acc = jnp.where(never, last, ys[n])
                for r in range(0, 128, 8):
                    w = wd_buf[i, pl.ds(128 * c + r, 8), pl.ds(128 * n, 128)].astype(F32)
                    acc = acc + w * hb[r:r + 8]
                last = ys[n] = acc
        for n in range(D // 128):
            y_acc[:, pl.ds(128 * n, 128)] = ys[n]

    def phase_b(i, carry):
        with _Scope("wf"):
            for c in f_copies(i):
                c.wait()
        for t in range(2):
            def emit_k(rh, ch, v, t=t):
                for p in range(NPAIR // 2):
                    pair = rh * (NPAIR // 2) + p
                    phi = _dual_softmax(v[64 * p:64 * p + 64])
                    z_acc[pair] += jnp.concatenate(phi, axis=0)
                    phik_buf.at[pair, 2 * t + ch][...] = _pack(jnp.concatenate(
                        [jnp.concatenate(phi[:8], axis=0), jnp.concatenate(phi[8:], axis=0)], axis=1))
            project_in(1, 2 * i + t, emit_k)
        ffn(i)
        prepare_weights(3, i)()
        for t in range(2):
            def emit_v(rh, ch, v, t=t):
                for p in range(0, NPAIR // 2, 2):
                    vt_buf.at[(rh * (NPAIR // 2) + p) // 2, 2 * t + ch][...] = _pack(jnp.concatenate(
                        [v[64 * p:64 * p + 64], v[64 * p + 64:64 * p + 128]], axis=1))
            project_in(2, 2 * i + t, emit_v)
        for p in range(NPAIR):
            vt = jnp.concatenate(
                [vt_buf[p // 2, u, :, pl.ds(128 * (p % 2), 128)] for u in range(4)], axis=1)
            phi = jnp.concatenate([jnp.concatenate(
                [phik_buf[p, u, :, pl.ds(128 * e, 128)] for e in range(2)], axis=0)
                for u in range(4)], axis=1)
            kv_acc[p] += _dot_nt(_unpack(vt), _unpack(phi))
        return carry

    with _Scope("phB"):
        lax.fori_loop(0, NB, phase_b, 0)

    y = _round_bf16(jnp.sum(y_acc[...], axis=0, keepdims=True))
    r_sel = _round_bf16(0.5 + 0.5 * jnp.tanh(0.5 * top[:, 0:1]))
    y = _round_bf16(y * r_sel)
    upd_buf[0] = jnp.zeros((8, D), F32)
    upd_buf[1] = jnp.where(lax.broadcasted_iota(jnp.int32, (8, D), 0) == idx % 8, y, 0.0)

    r_ = lax.broadcasted_iota(jnp.int32, (64, 128), 0)
    c_ = lax.broadcasted_iota(jnp.int32, (64, 128), 1)
    own = r_ // DH == c_ % 2
    for p in range(NPAIR // 2):
        kvb_buf.at[p][...] = _pack(jnp.concatenate(
            [jnp.where(own, kv_acc[p + NPAIR // 2 * u], 0.0) for u in range(2)], axis=1))
    for p in range(NPAIR):
        z_acc[p] = jnp.broadcast_to(jnp.sum(z_acc[p], axis=1, keepdims=True), (128, 128))

    def attend_pairs(j, p):
        odd = lax.broadcasted_iota(jnp.int32, (8, SUB), 0) % 2 == 1
        o = []
        for u in range(2):
            pair = p + NPAIR // 2 * u
            for ch in range(2):
                phi = _dual_softmax(pq_buf[j, ch, pl.ds(64 * pair, 64), :])
                den = _tree([phi[t] * z_acc[pair, pl.ds(8 * t, 8), :] for t in range(16)], jnp.add)
                rd = _recip(_allreduce(den, jnp.add) + 1e-6)
                rs = pltpu.roll(rd, 1, 0)
                r0 = jnp.where(odd, rs, rd)
                r1 = jnp.where(odd, rd, rs)
                num = _dot(_unpack(kvb_buf[p, :, pl.ds(128 * u, 128)]),
                           jnp.concatenate(phi, axis=0).astype(BF16))
                o.append(num * jnp.concatenate([r0] * 4 + [r1] * 4, axis=0))

        def store():
            os_buf.at[j % 2][pl.ds(32 * p, 32), :] = _pack(jnp.concatenate(_rhs_sums(*o), axis=1))
        return store

    def finish(j, rh, ch, v):
        cols = pl.ds(rh * HD, HD)
        s = v.T
        for r in range(0, SUB, 16):
            row0 = j * STEP + ch * SUB + r
            rows = pl.ds(row0, 16)
            x, xn = normalized(rows, cols)
            upd = jnp.concatenate([
                upd_buf[(idx // 8 == row0 // 8 + e).astype(jnp.int32), :, cols]
                for e in range(2)], axis=0)
            out_buf[rows, cols] = (x + s[r:r + 16] * _silu(xn + upd)).astype(BF16)

    later = Deferred()
    plan = {-1: (0,), 0: (1, 2), 1: (3,), 2: (4,), 3: (5,), 4: (6,), 5: (7,), 6: ()}

    def attend_between(j):
        def between(n):
            if n >= 0:
                later.tick()
            if j < NSTEP:
                for p in plan[n]:
                    later.add(1, attend_pairs(j, p))
        return between

    def out_product(j, n):
        rhs = os_buf[j % 2 + (zero if 0 else 0), :, pl.ds(SUB * n, SUB)]
        if 0 and j > 0:
            done = out_buf[pl.ds(pl.multiple_of(zero * 16, 16), 16), pl.ds(HD, 128)]
            rhs = jnp.concatenate([jnp.where(never, pltpu.bitcast(done, U32), rhs[:8]), rhs[8:]], axis=0)
        return _dot(_unpack(wo_sum[n]), _unpack(rhs))

    if True:
        attend_between(0)(-1)
        project_q(NSTEP - 1, attend_between(0))
    def barrier(name):
        with _Scope(name):
            pl.semaphore_signal(sem_order, 1)
            pl.semaphore_wait(sem_order, 1)

    last_blocks = [
        pltpu.make_async_copy(out_buf.at[blk], out_hbm.at[blk], sem_last.at[n])
        for n, blk in enumerate(
            (pl.ds(S - STEP + ch * SUB, SUB), pl.ds(rh * HD, HD))
            for rh, ch in ((1, 0), (0, 1), (0, 0), (1, 1)))]
    started = 0
    for j in range(NSTEP):
        def emit(rh, ch, v, j=j):
            later.add(1, lambda: finish(j, rh, ch, v))

        def side(n, j=j, attend=attend_between(j + 1)):
            nonlocal started
            attend(n)
            if n == 1 and j in FLUSH_AT:
                for jj in range(started, j):
                    o_copy(jj).start(priority=1)
                started = j
                barrier("fl%d" % j)
            if n == 4 and j == NSTEP - 1:
                for jj in range(started, j):
                    o_copy(jj).start(priority=1)
                for c in last_blocks[:2]:
                    c.start(priority=1)
                barrier("fl8")
        side(-1)
        _strassen(lambda n: out_product(j, n), emit, side)
    later.flush()
    for c in last_blocks[2:]:
        c.start(priority=1)
    with _Scope("wout"):
        for j in range(NSTEP - 1):
            o_copy(j).wait()
        for c in last_blocks:
            c.wait()


@jax.jit
def pallas_recurrent_scan__linear_kernel_hedgehog__moe_arch_mod__prompt_kernel(
    A_x: jax.Array,
    A_wqkv: jax.Array,
    A_w_phi: jax.Array,
    A_wo: jax.Array,
    B_x: jax.Array,
    B_w_r: jax.Array,
    B_w_gate: jax.Array,
    B_w_up: jax.Array,
    B_w_down: jax.Array,
):
    del B_x
    scratch = [
        pltpu.VMEM((S, D), BF16),
        pltpu.VMEM((NSTEP, 7, SUB // 2, HD), U32),
        pltpu.VMEM((2, S, 128), F32),
        pltpu.VMEM((4, D, D), BF16),
        pltpu.VMEM((3, 7, HD // 2, HD), U32),
        pltpu.VMEM((7, HD // 2, HD), U32),
        pltpu.VMEM((H * DH, DH), BF16),
        pltpu.VMEM((NG, 64, 256), U32),
        pltpu.VMEM((8, 128), BF16),
        pltpu.VMEM((NSTEP, 2, D, SUB), F32),
        pltpu.VMEM((NPAIR // 2, 4, 32, 256), U32),
        pltpu.VMEM((NPAIR, 4, 32, 256), U32),
        pltpu.VMEM((NPAIR, 64, 128), F32),
        pltpu.VMEM((NPAIR, 128, 128), F32),
        pltpu.VMEM((NPAIR // 2, 32, 256), U32),
        pltpu.VMEM((2, HD // 2, 7 * SUB), U32),
        pltpu.VMEM((NB, D, FC), BF16),
        pltpu.VMEM((NB, D, FC), BF16),
        pltpu.VMEM((NB, FC, D), BF16),
        pltpu.VMEM((D, 128), F32),
        pltpu.VMEM((8, D), F32),
        pltpu.VMEM((2, 8, D), F32),
        pltpu.VMEM((S, D), BF16),
        pltpu.SemaphoreType.DMA((len(X_CUTS) - 1,)),
        pltpu.SemaphoreType.DMA((2 * NG,)),
        pltpu.SemaphoreType.DMA((2,)),
        pltpu.SemaphoreType.DMA((2,)),
        pltpu.SemaphoreType.DMA((5 * NB,)),
        pltpu.SemaphoreType.DMA((NSTEP - 1,)),
        pltpu.SemaphoreType.DMA((4,)),
        pltpu.SemaphoreType.REGULAR,
    ]
    any_spec = pl.BlockSpec(memory_space=pl.ANY)
    flags = {}
    if 0:
        flags["XLA_TPU_FORCE_LP_LLO_SCHEDULER"] = True
    if 0:
        flags["XLA_TPU_EVENLY_DISTRIBUTE_CRITICAL_NODES"] = True
    out = pl.pallas_call(
        _kernel,
        out_shape=jax.ShapeDtypeStruct((S, D), BF16),
        in_specs=[any_spec] * 8,
        out_specs=any_spec,
        scratch_shapes=scratch,
        compiler_params=pltpu.CompilerParams(vmem_limit_bytes=120 * 2**20, flags=flags or None),
        name="hedgehog_mod",
    )(
        A_x.reshape(S, D),
        A_wqkv,
        A_w_phi.reshape(H * DH, DH),
        A_wo,
        B_w_r.reshape(8, 128),
        B_w_gate,
        B_w_up,
        B_w_down,
    )
    return out.reshape(1, S, D)
```

```python
import math

import jax
import jax.numpy as jnp
from jax import lax
import jax.experimental.pallas as pl
import jax.experimental.pallas.tpu as pltpu

S, D, H, DH, F = 2048, 1024, 32, 32, 3584
SUB = 128
STEP = 2 * SUB
NSTEP = S // STEP
NB = 4
FC = F // NB
HD = D // 2
NG = HD // 128
FLUSH_AT = [(3, 6), (6,), (5,), (4, 6)][0]
X_CUTS = (0, 1, 2, 4, 6, 10, 16)
GROUP = SUB // 16
NPAIR = H // 2
LOG2E = math.log2(math.e)
EPS = 1.0013580322265625e-05
F32, BF16, U32 = jnp.float32, jnp.bfloat16, jnp.uint32

NT_DIMS = (((1,), (1,)), ((), ()))


def _dot(a, b):
    return jnp.dot(a, b, preferred_element_type=F32)


def _dot_nt(a, b):
    return lax.dot_general(a, b, NT_DIMS, preferred_element_type=F32)


def _round_bf16(v):
    return v.astype(BF16).astype(F32)


def _pack(v):
    return pltpu.bitcast(v.astype(BF16), U32)


def _unpack(v):
    return pltpu.bitcast(v, BF16)


def _silu(t):
    h = 0.5 * t
    return h + h * jnp.tanh(h)


def _recip(d):
    r = pltpu.reciprocal(d, approx=True)
    return r * (2.0 - d * r)


def _allreduce(v, op):
    v = op(v, pltpu.roll(v, 4, 0))
    return op(v, pltpu.roll(v, 2, 0))


def _tree(vals, op):
    vals = list(vals)
    while len(vals) > 1:
        nxt = [op(vals[i], vals[i + 1]) for i in range(0, len(vals) - 1, 2)]
        if len(vals) % 2:
            nxt.append(vals[-1])
        vals = nxt
    return vals[0]


def _dual_softmax(p):
    ps = [p[8 * j:8 * j + 8] for j in range(8)]
    mx = _allreduce(_tree(ps, jnp.maximum), jnp.maximum)
    mn = _allreduce(_tree(ps, jnp.minimum), jnp.minimum)
    ep = [jnp.exp2(v - mx) for v in ps]
    en = [jnp.exp2(mn - v) for v in ps]
    rp = _recip(_allreduce(_tree(ep, jnp.add), jnp.add))
    rn = _recip(_allreduce(_tree(en, jnp.add), jnp.add))
    return [e * rp for e in ep] + [e * rn for e in en]


def _lhs_sums(a11, a12, a21, a22):
    return (a11 + a22, a21 + a22, a11, a22, a11 + a12, a21 - a11, a12 - a22)


def _rhs_sums(b11, b12, b21, b22):
    return (b11 + b22, b11, b12 - b22, b21 - b11, b22, b11 + b12, b21 + b22)


def _strassen(prod, emit, between=None):
    between = between or (lambda n: None)
    m2 = prod(1)
    between(0)
    m4 = prod(3)
    emit(1, 0, m2 + m4)
    between(1)
    m3 = prod(2)
    c22 = m3 - m2
    between(2)
    m5 = prod(4)
    emit(0, 1, m3 + m5)
    c11 = m4 - m5
    between(3)
    m1 = prod(0)
    c11 = c11 + m1
    c22 = c22 + m1
    between(4)
    emit(0, 0, c11 + prod(6))
    between(5)
    emit(1, 1, c22 + prod(5))
    between(6)


class _Scope:
    def __init__(self, name):
        self.s = jax.named_scope(name) if 0 else None

    def __enter__(self):
        if self.s:
            self.s.__enter__()

    def __exit__(self, *a):
        if self.s:
            self.s.__exit__(*a)


def _kernel(x_hbm, wqkv_hbm, wphi_hbm, wo_hbm, wr_hbm, wg_hbm, wu_hbm, wd_hbm,
            out_hbm,
            x_buf, xs_buf, stat_buf, w_raw, w_sum, wo_sum, wphi_buf, bd_buf, wr_buf,
            pq_buf, vt_buf, phik_buf, kv_acc, z_acc, kvb_buf, os_buf,
            wgu_buf, wd_buf, xb_buf, y_acc, upd_buf, out_buf,
            sem_x, sem_q, sem_w, sem_s, sem_f, sem_o, sem_last, sem_order):
    def x_copy(n):
        rows = pl.ds(X_CUTS[n] * SUB, (X_CUTS[n + 1] - X_CUTS[n]) * SUB)
        return pltpu.make_async_copy(x_hbm.at[rows], x_buf.at[rows], sem_x.at[n])

    def q_copy(rh, kh):
        blk = (pl.ds(kh * HD, HD), pl.ds(rh * HD, HD))
        return pltpu.make_async_copy(wqkv_hbm.at[blk], w_raw.at[0].at[blk], sem_q.at[2 * rh + kh])

    def w_copy(m):
        return pltpu.make_async_copy(wqkv_hbm.at[:, pl.ds(m * D, D)], w_raw.at[m], sem_w.at[m - 1])

    def f_copies(i):
        return (
            pltpu.make_async_copy(wg_hbm.at[:, pl.ds(i * FC, FC)], wgu_buf.at[i, :, pl.ds(0, FC)], sem_f.at[i]),
            pltpu.make_async_copy(wu_hbm.at[:, pl.ds(i * FC, FC)], wgu_buf.at[i, :, pl.ds(FC, FC)], sem_f.at[NB + i]),
            pltpu.make_async_copy(wd_hbm.at[pl.ds(i * FC, FC)], wd_buf.at[i], sem_f.at[2 * NB + i]),
        ) + tuple(
            pltpu.make_async_copy(wo_hbm.at[:, cols], w_raw.at[3, :, cols], sem_f.at[(3 + half) * NB + i])
            for half in range(2)
            for cols in [pl.ds(pl.multiple_of(128 * (i + NG * half), 128), 128)])

    def o_copy(j):
        return pltpu.make_async_copy(
            out_buf.at[pl.ds(j * STEP, STEP)], out_hbm.at[pl.ds(j * STEP, STEP)], sem_o.at[j])

    wphi_copy = pltpu.make_async_copy(wphi_hbm, wphi_buf, sem_s.at[0])
    wr_copy = pltpu.make_async_copy(wr_hbm, wr_buf, sem_s.at[1])

    def fold_matrix(g):
        r = lax.broadcasted_iota(jnp.int32, (128, DH), 0)
        f = lax.broadcasted_iota(jnp.int32, (128, DH), 1)
        sel = jnp.where((r % 64) // 2 == f, 1.0, 0.0).astype(BF16)
        t = _dot_nt(sel, wphi_buf[pl.ds(128 * g, 128), :])
        r = lax.broadcasted_iota(jnp.int32, (128, 128), 0)
        c = lax.broadcasted_iota(jnp.int32, (128, 128), 1)
        return jnp.where(2 * (r // 64) + r % 2 == c // DH, t, 0.0)

    def prepare_weights(m, g):
        def block(half, k0):
            w = w_raw[m, pl.ds(k0, 256), pl.ds(pl.multiple_of(128 * (g + NG * half), 128), 128)]
            if m < 2:
                return _dot_nt(_unpack(bd_buf[g, :, pl.ds(128 * half, 128)]), w) * LOG2E
            return w.T.astype(F32)

        blocks = {k0: (block(0, k0), block(0, HD + k0), block(1, k0), block(1, HD + k0))
                  for k0 in range(0, HD, 256)}

        def store():
            dst = wo_sum if m == 3 else w_sum.at[m]
            for k0, quad in blocks.items():
                for n, v in enumerate(_lhs_sums(*quad)):
                    dst.at[n][pl.ds(pl.multiple_of(64 * g, 64), 64), pl.ds(k0, 256)] = _pack(v)
        return store

    lane16 = lax.broadcasted_iota(jnp.int32, (16, 128), 1)
    scores = [jnp.full((16, 128), -jnp.inf, F32)]

    def token_stats(j, never16, halves=(0, 1)):
        wr = wr_buf[...].astype(F32)
        wrow = jnp.concatenate(
            [jnp.broadcast_to(wr[c:c + 1], (16, 128)) for c in range(8)], axis=1)
        last = None
        for t0 in [(2 * j + half) * GROUP for half in halves]:
            sq = dot = jnp.zeros((16, 128), F32)
            for t in range(t0, t0 + GROUP):
                rows = pl.ds(16 * t, 16)
                x = x_buf[rows, :].astype(F32)
                if last is not None:
                    x = jnp.concatenate([jnp.where(never16, last, x[:, :128]), x[:, 128:]], axis=1)
                mean = jnp.sum(x, axis=1, keepdims=True) * (1.0 / D)
                stat_buf[0, rows, :] = jnp.broadcast_to(mean, (16, 128))
                c = x - mean
                sq = jnp.where(lane16 == t, jnp.sum(c * c, axis=1, keepdims=True), sq)
                dot = jnp.where(lane16 == t, jnp.sum(c * wrow, axis=1, keepdims=True), dot)
                if never16 is not None and t % 2 == 0:
                    last = sq
                yield
            inv = 1.0 / _round_bf16(jnp.sqrt(_round_bf16(_round_bf16(sq * (1.0 / D)) + EPS)))
            mine = (lane16 >= t0) & (lane16 < t0 + GROUP)
            score = _round_bf16(dot * inv)
            scores[0] = jnp.where(mine & (score == score), score, scores[0])
            for t in range(t0, t0 + GROUP):
                stat_buf[1, pl.ds(16 * t, 16), :] = jnp.broadcast_to(inv[:, t:t + 1], (16, 128))
        yield

    def advance(gen, count):
        for _ in range(count):
            next(gen, None)

    def normalized(rows, cols=slice(None), token=None):
        x = x_buf[rows, cols].astype(F32)
        reps = x.shape[1] // 128
        mean = stat_buf[0, rows, :]
        if token is not None:
            mean = jnp.where(never16, token, mean)
        mean = jnp.concatenate([mean] * reps, axis=1)
        inv = jnp.concatenate([stat_buf[1, rows, :]] * reps, axis=1)
        return x, (x - mean) * inv

    def token_sums(j, which=range(7)):
        for r in range(0, SUB, 16):
            a = normalized(pl.ds(j * STEP + r, 16))[1]
            b = normalized(pl.ds(j * STEP + SUB + r, 16))[1] if 0 in which else a
            for n, v in enumerate(_rhs_sums(a[:, :HD], b[:, :HD], a[:, HD:], b[:, HD:])):
                if n in which:
                    xs_buf.at[j, n][pl.ds(r // 2, 8), :] = _pack(v)
            yield

    def project_in(m, j, emit, between=None):
        _strassen(lambda n: _dot_nt(_unpack(w_sum[m, n]), _unpack(xs_buf[j, n])), emit, between)

    def project_q(j, between=None, m=0):
        def emit(rh, ch, v):
            pq_buf[j, ch, pl.ds(rh * HD, HD), :] = v
        project_in(m, j, emit, between)

    class Deferred:
        def __init__(self):
            self.now = 0
            self.items = []

        def add(self, delay, fn):
            self.items.append((self.now + delay, fn))

        def tick(self):
            self.now += 1
            due = [fn for t, fn in self.items if t <= self.now]
            self.items = [(t, fn) for t, fn in self.items if t > self.now]
            for fn in due:
                fn()

        def flush(self):
            for _, fn in self.items:
                fn()
            self.items = []

    def start_in_order(copies):
        for c in copies:
            c.start(priority=0)
            pl.semaphore_signal(sem_order, 1)
            pl.semaphore_wait(sem_order, 1)

    start_in_order(
        [wr_copy, x_copy(0), wphi_copy, q_copy(1, 1), x_copy(1), q_copy(1, 0), q_copy(0, 0),
         x_copy(2), q_copy(0, 1), x_copy(3), x_copy(4), w_copy(2), w_copy(1), x_copy(5)]
        + list(f_copies(0)))
    kv_acc[...] = jnp.zeros(kv_acc.shape, F32)
    z_acc[...] = jnp.zeros(z_acc.shape, F32)
    y_acc[...] = jnp.zeros(y_acc.shape, F32)
    with _Scope("wr"):
        wr_copy.wait()
    with _Scope("wx0"):
        x_copy(0).wait()
    advance(token_stats(0, None, (0,)), STEP)
    never = stat_buf[1, pl.ds(0, 8), :] < 0.0
    never16 = jnp.concatenate([never, never], axis=0)
    never2 = jnp.concatenate([never, never], axis=1)
    zero = never.astype(jnp.int32)[0, 0]
    advance(token_sums(0, (1, 3)), STEP)
    with _Scope("wphi"):
        wphi_copy.wait()
    for g in range(NG):
        bd_buf.at[g][...] = _pack(jnp.concatenate([fold_matrix(g), fold_matrix(g + NG)], axis=1))

    def quadrant(rh, kh):
        with _Scope("wq%d%d" % (rh, kh)):
            q_copy(rh, kh).wait()
        return jnp.concatenate([
            _dot_nt(_unpack(bd_buf[g, :, pl.ds(128 * rh, 128)]),
                    w_raw[0, pl.ds(kh * HD, HD), pl.ds(rh * HD + 128 * g, 128)]) * LOG2E
            for g in range(NG)], axis=0)

    def first_product(n, lhs):
        lhs = _pack(lhs)
        w_sum.at[0, n][...] = lhs
        return _dot_nt(_unpack(lhs), _unpack(xs_buf[0, n]))

    a22 = quadrant(1, 1)
    m4 = first_product(3, a22)
    x_copy(1).wait()
    a21 = quadrant(1, 0)
    advance(token_stats(0, None, (1,)), STEP)
    advance(token_sums(0, (0, 2, 4, 5, 6)), STEP)
    m2 = first_product(1, a21 + a22)
    pq_buf[0, 0, pl.ds(HD, HD), :] = m2 + m4
    a11 = quadrant(0, 0)
    m3 = first_product(2, a11)
    m1 = first_product(0, a11 + a22)
    pq_buf[0, 1, pl.ds(HD, HD), :] = m3 - m2 + m1 + first_product(5, a21 - a11)
    with _Scope("wx1"):
        x_copy(2).wait()
    a12 = quadrant(0, 1)
    advance(token_stats(1, never16 if 0 else None), STEP)
    m5 = first_product(4, a11 + a12)
    pq_buf[0, 1, pl.ds(0, HD), :] = m3 + m5
    pq_buf[0, 0, pl.ds(0, HD), :] = m4 + m1 - m5 + first_product(6, a12 - a22)
    advance(token_sums(1), STEP)

    stat_plans = [(4, 4, 4, 5, 0, 0, 0), (3, 3, 3, 3, 2, 3, 0), (4, 3, 3, 3, 4, 0, 0), (3, 3, 2, 3, 2, 2, 2)]
    sum_plans = [(0,) * 7, (2, 1, 1, 1, 1, 1, 1), (1, 1, 2, 1, 2, 1, 0), (2, 2, 2, 2, 0, 0, 0), (0, 0, 0, 2, 2, 2, 2)]
    later = Deferred()
    for j in range(1, NSTEP - 1):
        if j in (1, 2):
            with _Scope("wx2"):
                x_copy(j + 2).wait()
        if j == 4:
            with _Scope("wkv"):
                w_copy(2).wait()
                w_copy(1).wait()
                x_copy(5).wait()
        ahead = 0 and j > 0
        near = token_stats(j + 1, never16) if not ahead or j == 1 else iter(())
        far = token_stats(j + 2, never16) if ahead and j + 2 < NSTEP else iter(())
        sums = token_sums(j + 1)

        def side(n, j=j, near=near, far=far, sums=sums, ahead=ahead):
            later.tick()
            advance(near, stat_plans[0][n])
            advance(far, stat_plans[3][n])
            if ahead and j > 1:
                advance(sums, sum_plans[1][n])
            t = 7 * (j - 4) + n
            if t >= 0 and t % 5 == 0 and t // 5 < NG:
                later.add(2, prepare_weights(1, t // 5))
            if t >= 0 and t % 5 == 2 and t // 5 < NG:
                later.add(2, prepare_weights(2, t // 5))
        project_q(j, side)
        for gen in (near, far, sums):
            advance(gen, STEP)
    later.flush()

    top = jnp.max(jnp.max(scores[0], axis=0, keepdims=True), axis=1, keepdims=True)
    token = (16 * lane16 + lax.broadcasted_iota(jnp.int32, (16, 128), 0)).astype(F32)
    cand = jnp.where(scores[0] == top, token, float(S))
    idx = jnp.min(jnp.min(cand, axis=0, keepdims=True), axis=1, keepdims=True).astype(jnp.int32)[0, 0]
    idx = jnp.clip(idx, 0, S - 1)
    slab = pl.ds(pl.multiple_of((idx // 16) * 16, 16), 16)
    pick = lax.broadcasted_iota(jnp.int32, (16, D), 0) == idx % 16
    x_sel = jnp.sum(jnp.where(pick, _round_bf16(normalized(slab)[1]), 0.0), axis=0, keepdims=True)
    for c in range(D // 128):
        xb_buf[pl.ds(128 * c, 128), :] = jnp.broadcast_to(
            x_sel[:, 128 * c:128 * c + 128], (128, 128)).T

    def after(token, v):
        top = jnp.where(never, token, v[:8, :128])
        if v.shape[1] > 128:
            top = jnp.concatenate([top, v[:8, 128:]], axis=1)
        return jnp.concatenate([top, v[8:]], axis=0)

    def paced(acc, step):
        if not 0 or step % 0 != 0 - 1:
            return acc
        slow = pltpu.reciprocal(acc[:, :128], approx=True)
        return jnp.where(never2, jnp.concatenate([slow, slow], axis=1), acc)

    def ffn(i):
        last = None
        act = []
        for c in range(0, 2 * FC, 256):
            acc = jnp.zeros((8, 256), F32)
            if last is not None:
                acc = jnp.where(never2, last, acc)
            for r in range(0, D, 8):
                xb = xb_buf[pl.ds(r, 8), :]
                w = wgu_buf[i, pl.ds(r, 8), pl.ds(c, 256)].astype(F32)
                acc = paced(acc + w * jnp.concatenate([xb, xb], axis=1), r // 8)
            last = acc
            act.append(_round_bf16(jnp.sum(acc, axis=0, keepdims=True)))
        act = jnp.concatenate(act, axis=1)
        h = _round_bf16(_round_bf16(_silu(act[:, :FC])) * act[:, FC:])
        ys = [y_acc[:, pl.ds(n, 256)] for n in range(0, D, 256)]
        for c in range(0, FC, 128):
            hb = jnp.broadcast_to(h[:, c:c + 128], (128, 128)).T
            for n in range(D // 256):
                acc = jnp.where(never2, last, ys[n])
                for r in range(0, 128, 8):
                    w = wd_buf[i, pl.ds(c + r, 8), pl.ds(256 * n, 256)].astype(F32)
                    acc = paced(acc + w * jnp.concatenate([hb[r:r + 8]] * 2, axis=1), r // 8)
                last = ys[n] = acc
        for n in range(D // 256):
            y_acc[:, pl.ds(256 * n, 256)] = ys[n]
        return last

    def phase_b(i, carry):
        with _Scope("wf"):
            for c in f_copies(i):
                c.wait()

        @pl.when(i + 1 < NB)
        def _():
            start_in_order(f_copies(i + 1))

        for t in range(2):
            def emit_k(rh, ch, v, t=t):
                for p in range(NPAIR // 2):
                    pair = rh * (NPAIR // 2) + p
                    phi = _dual_softmax(v[64 * p:64 * p + 64])
                    z_acc[pair] += jnp.concatenate(phi, axis=0)
                    phik_buf.at[pair, 2 * t + ch][...] = _pack(jnp.concatenate(
                        [jnp.concatenate(phi[:8], axis=0), jnp.concatenate(phi[8:], axis=0)], axis=1))
            project_in(1, 2 * i + t, emit_k)
        prepare_weights(3, i)()
        done = ffn(i)
        for t in range(2):
            def emit_v(rh, ch, v, t=t):
                for p in range(0, NPAIR // 2, 2):
                    vt_buf.at[(rh * (NPAIR // 2) + p) // 2, 2 * t + ch][...] = _pack(jnp.concatenate(
                        [v[64 * p:64 * p + 64], v[64 * p + 64:64 * p + 128]], axis=1))

            def product(n, t=t):
                rhs = xs_buf[2 * i + t, n]
                if (t, n) == (0, 6) and 1:
                    rhs = after(wo_sum[0, pl.ds(0, 8), pl.ds(0, 128)], rhs)
                if (t, n) == (1, 5) and 0:
                    rhs = after(pltpu.bitcast(done[:, :128], U32), rhs)
                return _dot_nt(_unpack(w_sum[2, n]), _unpack(rhs))
            _strassen(product, emit_v)
        for p in range(NPAIR):
            vt = jnp.concatenate(
                [vt_buf[p // 2, u, :, pl.ds(128 * (p % 2), 128)] for u in range(4)], axis=1)
            phi = jnp.concatenate([jnp.concatenate(
                [phik_buf[p, u, :, pl.ds(128 * e, 128)] for e in range(2)], axis=0)
                for u in range(4)], axis=1)
            kv_acc[p] += _dot_nt(_unpack(vt), _unpack(phi))
        return carry

    def keep_alive():
        for ref in (pq_buf.at[0, 0], xs_buf.at[0, 0], w_sum.at[0, 0], stat_buf.at[0], xb_buf, kv_acc.at[0], z_acc.at[0], y_acc, wo_sum.at[0]):
            c = pltpu.make_async_copy(ref, ref, sem_s.at[0])
            c.start()
            c.wait()

    if 0 == 1:
        for c in f_copies(0):
            c.wait()
        return keep_alive()
    if 0 in (0, 2):
        with _Scope("phB"):
            lax.fori_loop(0, NB, phase_b, 0)
    if 0 == 2:
        return keep_alive()

    y = _round_bf16(jnp.sum(y_acc[...], axis=0, keepdims=True))
    r_sel = _round_bf16(0.5 + 0.5 * jnp.tanh(0.5 * top))
    y = _round_bf16(y * r_sel)
    upd_buf[0] = jnp.zeros((8, D), F32)
    upd_buf[1] = jnp.where(lax.broadcasted_iota(jnp.int32, (8, D), 0) == idx % 8, y, 0.0)

    r_ = lax.broadcasted_iota(jnp.int32, (64, 128), 0)
    c_ = lax.broadcasted_iota(jnp.int32, (64, 128), 1)
    own = r_ // DH == c_ % 2
    for p in range(NPAIR // 2):
        kvb_buf.at[p][...] = _pack(jnp.concatenate(
            [jnp.where(own, kv_acc[p + NPAIR // 2 * u], 0.0) for u in range(2)], axis=1))
    for p in range(NPAIR):
        z_acc[p] = jnp.broadcast_to(jnp.sum(z_acc[p], axis=1, keepdims=True), (128, 128))

    recent = []

    def attend_pairs(j, p):
        odd = lax.broadcasted_iota(jnp.int32, (8, SUB), 0) % 2 == 1
        o = []
        for u in range(2):
            pair = p + NPAIR // 2 * u
            for ch in range(2):
                logits = pq_buf[j, ch, pl.ds(64 * pair, 64), :]
                if 0 and len(recent) >= 0:
                    logits = after(recent[-0], logits)
                phi = _dual_softmax(logits)
                den = _tree([phi[t] * z_acc[pair, pl.ds(8 * t, 8), :] for t in range(16)], jnp.add)
                rd = _recip(_allreduce(den, jnp.add) + 1e-6)
                rs = pltpu.roll(rd, 1, 0)
                r0 = jnp.where(odd, rs, rd)
                r1 = jnp.where(odd, rd, rs)
                num = _dot(_unpack(kvb_buf[p, :, pl.ds(128 * u, 128)]),
                           jnp.concatenate(phi, axis=0).astype(BF16))
                o.append(num * jnp.concatenate([r0] * 4 + [r1] * 4, axis=0))

        def store():
            os_buf.at[j % 2][pl.ds(32 * p, 32), :] = _pack(jnp.concatenate(_rhs_sums(*o), axis=1))
            if 0 == 2 and j > 0:
                seen = os_buf[j % 2 + zero, pl.ds(pl.multiple_of(zero * 8 + 32 * p, 8), 8),
                              pl.ds(pl.multiple_of(zero * 128, 128), 128)]
                later.add(2, lambda: due.append(seen))
        return store

    last_blocks = {
        (rh, ch): pltpu.make_async_copy(out_buf.at[blk], out_hbm.at[blk], sem_last.at[2 * rh + ch])
        for rh in range(2) for ch in range(2)
        for blk in [(pl.ds(S - STEP + ch * SUB, SUB), pl.ds(rh * HD, HD))]}

    def finish(j, rh, ch, v):
        cols = pl.ds(rh * HD, HD)
        s = v.T
        for r in range(0, SUB, 16):
            row0 = j * STEP + ch * SUB + r
            rows = pl.ds(row0, 16)
            x, xn = normalized(rows, cols, s[r:r + 16, :128] if 0 else None)
            upd = jnp.concatenate([
                upd_buf[(idx // 8 == row0 // 8 + e).astype(jnp.int32), :, cols]
                for e in range(2)], axis=0)
            out_buf[rows, cols] = (x + s[r:r + 16] * _silu(xn + upd)).astype(BF16)
        if j == NSTEP - 1:
            last_blocks[rh, ch].start(priority=0)
        elif (rh, ch) == (1, 1):
            o_copy(j).start(priority=0)
        seen = out_buf[pl.ds(pl.multiple_of(zero * 16, 16), 16),
                       pl.ds(pl.multiple_of(zero * 128 + HD, 128), 128)]
        if 1 or (rh, ch) == (1, 0):
            later.add(3, lambda: due.append(pltpu.bitcast(seen, U32)))

    later = Deferred()
    due = []
    plan = {-1: (0,), 0: (1, 2), 1: (3,), 2: (4,), 3: (5,), 4: (6,), 5: (7,), 6: ()}

    def attend_between(j):
        def between(n):
            if n >= 0:
                later.tick()
            if j < NSTEP:
                for p in plan[n]:
                    later.add(1, attend_pairs(j, p))
        return between

    attend_between(0)(-1)
    project_q(NSTEP - 1, attend_between(0))
    for j in range(NSTEP):
        def emit(rh, ch, v, j=j):
            if j == NSTEP - 1 and 1:
                finish(j, rh, ch, v)
            else:
                later.add(1, lambda: finish(j, rh, ch, v))

        def product(n, j=j):
            rhs = os_buf[j % 2 + (zero if 0 == 1 else 0), :, pl.ds(SUB * n, SUB)]
            while due:
                rhs = after(due.pop(), rhs)
            m = _dot(_unpack(wo_sum[n]), _unpack(rhs))
            recent.append(m[:8])
            return m
        attend = attend_between(j + 1)
        attend(-1)
        _strassen(product, emit, attend)
    later.flush()
    with _Scope("wout"):
        for j in range(NSTEP - 1):
            o_copy(j).wait()
        for c in last_blocks.values():
            c.wait()


@jax.jit
def pallas_recurrent_scan__linear_kernel_hedgehog__moe_arch_mod__prompt_kernel(
    A_x: jax.Array,
    A_wqkv: jax.Array,
    A_w_phi: jax.Array,
    A_wo: jax.Array,
    B_x: jax.Array,
    B_w_r: jax.Array,
    B_w_gate: jax.Array,
    B_w_up: jax.Array,
    B_w_down: jax.Array,
):
    del B_x
    scratch = [
        pltpu.VMEM((S, D), BF16),
        pltpu.VMEM((NSTEP, 7, SUB // 2, HD), U32),
        pltpu.VMEM((2, S, 128), F32),
        pltpu.VMEM((4, D, D), BF16),
        pltpu.VMEM((3, 7, HD // 2, HD), U32),
        pltpu.VMEM((7, HD // 2, HD), U32),
        pltpu.VMEM((H * DH, DH), BF16),
        pltpu.VMEM((NG, 64, 256), U32),
        pltpu.VMEM((8, 128), BF16),
        pltpu.VMEM((NSTEP, 2, D, SUB), F32),
        pltpu.VMEM((NPAIR // 2, 4, 32, 256), U32),
        pltpu.VMEM((NPAIR, 4, 32, 256), U32),
        pltpu.VMEM((NPAIR, 64, 128), F32),
        pltpu.VMEM((NPAIR, 128, 128), F32),
        pltpu.VMEM((NPAIR // 2, 32, 256), U32),
        pltpu.VMEM((2, HD // 2, 7 * SUB), U32),
        pltpu.VMEM((NB, D, 2 * FC), BF16),
        pltpu.VMEM((NB, FC, D), BF16),
        pltpu.VMEM((D, 128), F32),
        pltpu.VMEM((8, D), F32),
        pltpu.VMEM((2, 8, D), F32),
        pltpu.VMEM((S, D), BF16),
        pltpu.SemaphoreType.DMA((len(X_CUTS) - 1,)),
        pltpu.SemaphoreType.DMA((4,)),
        pltpu.SemaphoreType.DMA((2,)),
        pltpu.SemaphoreType.DMA((2,)),
        pltpu.SemaphoreType.DMA((5 * NB,)),
        pltpu.SemaphoreType.DMA((NSTEP - 1,)),
        pltpu.SemaphoreType.DMA((4,)),
        pltpu.SemaphoreType.REGULAR,
    ]
    any_spec = pl.BlockSpec(memory_space=pl.ANY)
    flags = {}
    if 0:
        flags["XLA_TPU_FORCE_LP_LLO_SCHEDULER"] = True
    if 0:
        flags["XLA_TPU_EVENLY_DISTRIBUTE_CRITICAL_NODES"] = True
    out = pl.pallas_call(
        _kernel,
        out_shape=jax.ShapeDtypeStruct((S, D), BF16),
        in_specs=[any_spec] * 8,
        out_specs=any_spec,
        scratch_shapes=scratch,
        compiler_params=pltpu.CompilerParams(vmem_limit_bytes=120 * 2**20, flags=flags or None),
        name="hedgehog_mod",
    )(
        A_x.reshape(S, D),
        A_wqkv,
        A_w_phi.reshape(H * DH, DH),
        A_wo,
        B_w_r.reshape(8, 128),
        B_w_gate,
        B_w_up,
        B_w_down,
    )
    return out.reshape(1, S, D)
```

```python
import math

import jax
import jax.numpy as jnp
from jax import lax
import jax.experimental.pallas as pl
import jax.experimental.pallas.tpu as pltpu

S, D, H, DH, F = 2048, 1024, 32, 32, 3584
SUB = 128
STEP = 2 * SUB
NSTEP = S // STEP
NB = 4
FC = F // NB
HD = D // 2
NG = HD // 128
FLUSH_AT = [(3, 6), (6,), (5,), (4, 6)][0]
X_CUTS = (0, 1, 2, 3, 4, 8, 12, 16)
GROUP = SUB // 16
NPAIR = H // 2
LOG2E = math.log2(math.e)
EPS = 1.0013580322265625e-05
F32, BF16, U32 = jnp.float32, jnp.bfloat16, jnp.uint32

NT_DIMS = (((1,), (1,)), ((), ()))


def _dot(a, b):
    return jnp.dot(a, b, preferred_element_type=F32)


def _dot_nt(a, b):
    return lax.dot_general(a, b, NT_DIMS, preferred_element_type=F32)


def _round_bf16(v):
    return v.astype(BF16).astype(F32)


def _pack(v):
    return pltpu.bitcast(v.astype(BF16), U32)


def _unpack(v):
    return pltpu.bitcast(v, BF16)


def _silu(t):
    h = 0.5 * t
    return h + h * jnp.tanh(h)


def _recip(d):
    r = pltpu.reciprocal(d, approx=True)
    return r * (2.0 - d * r) if 0 else r


def _allreduce(v, op):
    v = op(v, pltpu.roll(v, 4, 0))
    return op(v, pltpu.roll(v, 2, 0))


def _tree(vals, op):
    vals = list(vals)
    while len(vals) > 1:
        nxt = [op(vals[i], vals[i + 1]) for i in range(0, len(vals) - 1, 2)]
        if len(vals) % 2:
            nxt.append(vals[-1])
        vals = nxt
    return vals[0]


def _dual_softmax(p):
    ps = [p[8 * j:8 * j + 8] for j in range(8)]
    mx = _allreduce(_tree(ps, jnp.maximum), jnp.maximum)
    mn = _allreduce(_tree(ps, jnp.minimum), jnp.minimum)
    ep = [jnp.exp2(v - mx) for v in ps]
    en = [jnp.exp2(mn - v) for v in ps]
    rp = _recip(_allreduce(_tree(ep, jnp.add), jnp.add))
    rn = _recip(_allreduce(_tree(en, jnp.add), jnp.add))
    return [e * rp for e in ep] + [e * rn for e in en]


def _lhs_sums(a11, a12, a21, a22):
    return (a11 + a22, a21 + a22, a11, a22, a11 + a12, a21 - a11, a12 - a22)


def _rhs_sums(b11, b12, b21, b22):
    return (b11 + b22, b11, b12 - b22, b21 - b11, b22, b11 + b12, b21 + b22)


def _strassen(prod, emit, between=None):
    between = between or (lambda n: None)
    m2 = prod(1)
    between(0)
    m4 = prod(3)
    emit(1, 0, m2 + m4)
    between(1)
    m3 = prod(2)
    c22 = m3 - m2
    between(2)
    m5 = prod(4)
    emit(0, 1, m3 + m5)
    c11 = m4 - m5
    between(3)
    m1 = prod(0)
    c11 = c11 + m1
    c22 = c22 + m1
    between(4)
    emit(0, 0, c11 + prod(6))
    between(5)
    emit(1, 1, c22 + prod(5))
    between(6)


class _Scope:
    def __init__(self, name):
        self.s = jax.named_scope(name) if 0 else None

    def __enter__(self):
        if self.s:
            self.s.__enter__()

    def __exit__(self, *a):
        if self.s:
            self.s.__exit__(*a)


def _kernel(x_hbm, wqkv_hbm, wphi_hbm, wo_hbm, wr_hbm, wg_hbm, wu_hbm, wd_hbm,
            out_hbm,
            x_buf, xs_buf, stat_buf, w_raw, w_sum, wo_sum, wphi_buf, bd_buf, wr_buf,
            pq_buf, vt_buf, phik_buf, kv_acc, z_acc, kvb_buf, os_buf,
            wgu_buf, wd_buf, xb_buf, y_acc, upd_buf, gate_buf, out_buf,
            sem_x, sem_q, sem_w, sem_s, sem_f, sem_o, sem_last, sem_order):
    def x_copy(n):
        rows = pl.ds(X_CUTS[n] * SUB, (X_CUTS[n + 1] - X_CUTS[n]) * SUB)
        return pltpu.make_async_copy(x_hbm.at[rows], x_buf.at[rows], sem_x.at[n])

    def q_copy(rh, kh):
        blk = (pl.ds(kh * HD, HD), pl.ds(rh * HD, HD))
        return pltpu.make_async_copy(wqkv_hbm.at[blk], w_raw.at[0].at[blk], sem_q.at[2 * rh + kh])

    def w_copy(m):
        return pltpu.make_async_copy(wqkv_hbm.at[:, pl.ds(m * D, D)], w_raw.at[m], sem_w.at[m - 1])

    def f_copies(i):
        return (
            pltpu.make_async_copy(wg_hbm.at[:, pl.ds(i * FC, FC)], wgu_buf.at[i, :, pl.ds(0, FC)], sem_f.at[i]),
            pltpu.make_async_copy(wu_hbm.at[:, pl.ds(i * FC, FC)], wgu_buf.at[i, :, pl.ds(FC, FC)], sem_f.at[NB + i]),
            pltpu.make_async_copy(wd_hbm.at[pl.ds(i * FC, FC)], wd_buf.at[i], sem_f.at[2 * NB + i]),
        ) + tuple(
            pltpu.make_async_copy(wo_hbm.at[:, cols], w_raw.at[3, :, cols], sem_f.at[(3 + half) * NB + i])
            for half in range(2)
            for cols in [pl.ds(pl.multiple_of(128 * (i + NG * half), 128), 128)])

    def o_copy(j):
        return pltpu.make_async_copy(
            out_buf.at[pl.ds(j * STEP, STEP)], out_hbm.at[pl.ds(j * STEP, STEP)], sem_o.at[j])

    wphi_copy = pltpu.make_async_copy(wphi_hbm, wphi_buf, sem_s.at[0])
    wr_copy = pltpu.make_async_copy(wr_hbm, wr_buf, sem_s.at[1])

    def fold_matrix(g):
        r = lax.broadcasted_iota(jnp.int32, (128, DH), 0)
        f = lax.broadcasted_iota(jnp.int32, (128, DH), 1)
        sel = jnp.where((r % 64) // 2 == f, 1.0, 0.0).astype(BF16)
        t = _dot_nt(sel, wphi_buf[pl.ds(128 * g, 128), :])
        r = lax.broadcasted_iota(jnp.int32, (128, 128), 0)
        c = lax.broadcasted_iota(jnp.int32, (128, 128), 1)
        return jnp.where(2 * (r // 64) + r % 2 == c // DH, t * LOG2E, 0.0)

    def prepare_weights(m, g):
        def block(half, k0):
            w = w_raw[m, pl.ds(k0, 256), pl.ds(pl.multiple_of(128 * (g + NG * half), 128), 128)]
            if m < 2:
                return _dot_nt(_unpack(bd_buf[g, :, pl.ds(128 * half, 128)]), w)
            return w.T.astype(F32)

        blocks = {k0: (block(0, k0), block(0, HD + k0), block(1, k0), block(1, HD + k0))
                  for k0 in range(0, HD, 256)}

        def store():
            dst = wo_sum if m == 3 else w_sum.at[m]
            for k0, quad in blocks.items():
                for n, v in enumerate(_lhs_sums(*quad)):
                    dst.at[n][pl.ds(pl.multiple_of(64 * g, 64), 64), pl.ds(k0, 256)] = _pack(v)
        return store

    lane16 = lax.broadcasted_iota(jnp.int32, (16, 128), 1)
    scores = [jnp.full((16, 128), -jnp.inf, F32)]

    def token_stats(j, never16, halves=(0, 1)):
        wr = wr_buf[...].astype(F32)
        wrow = jnp.concatenate(
            [jnp.broadcast_to(wr[c:c + 1], (16, 128)) for c in range(8)], axis=1)
        last = None
        for t0 in [(2 * j + half) * GROUP for half in halves]:
            sq = dot = jnp.zeros((16, 128), F32)
            for t in range(t0, t0 + GROUP):
                rows = pl.ds(16 * t, 16)
                x = x_buf[rows, :].astype(F32)
                if last is not None:
                    x = jnp.concatenate([jnp.where(never16, last, x[:, :128]), x[:, 128:]], axis=1)
                mean = jnp.sum(x, axis=1, keepdims=True) * (1.0 / D)
                stat_buf[0, rows, :] = jnp.broadcast_to(mean, (16, 128))
                c = x - mean
                sq = jnp.where(lane16 == t, jnp.sum(c * c, axis=1, keepdims=True), sq)
                dot = jnp.where(lane16 == t, jnp.sum(c * wrow, axis=1, keepdims=True), dot)
                if never16 is not None and t % 2 == 0:
                    last = sq
                yield
            inv = 1.0 / _round_bf16(jnp.sqrt(_round_bf16(_round_bf16(sq * (1.0 / D)) + EPS)))
            mine = (lane16 >= t0) & (lane16 < t0 + GROUP)
            score = _round_bf16(dot * inv)
            scores[0] = jnp.where(mine & (score == score), score, scores[0])
            for t in range(t0, t0 + GROUP):
                stat_buf[1, pl.ds(16 * t, 16), :] = jnp.broadcast_to(inv[:, t:t + 1], (16, 128))
        yield

    def advance(gen, count):
        for _ in range(count):
            next(gen, None)

    def normalized(rows, cols=slice(None), token=None):
        x = x_buf[rows, cols].astype(F32)
        reps = x.shape[1] // 128
        mean = stat_buf[0, rows, :]
        if token is not None:
            mean = jnp.where(never16, token, mean)
        mean = jnp.concatenate([mean] * reps, axis=1)
        inv = jnp.concatenate([stat_buf[1, rows, :]] * reps, axis=1)
        return x, (x - mean) * inv

    def token_sums(j, which=range(7)):
        for r in range(0, SUB, 16):
            a = normalized(pl.ds(j * STEP + r, 16))[1]
            b = normalized(pl.ds(j * STEP + SUB + r, 16))[1] if 0 in which else a
            for n, v in enumerate(_rhs_sums(a[:, :HD], b[:, :HD], a[:, HD:], b[:, HD:])):
                if n in which:
                    xs_buf.at[j, n][pl.ds(r // 2, 8), :] = _pack(v)
            yield

    def after(token, v):
        top = jnp.where(never, token, v[:8, :128])
        if v.shape[1] > 128:
            top = jnp.concatenate([top, v[:8, 128:]], axis=1)
        return jnp.concatenate([top, v[8:]], axis=0)

    due = []

    def when_due(v):
        while due:
            v = after(due.pop(), v)
        return v

    def written(ref):
        return ref[pl.ds(pl.multiple_of(zero * 16, 16), 16 if ref.dtype == BF16 else 8),
                   pl.ds(pl.multiple_of(zero * 128, 128), 128)]

    def project_in(m, j, emit, between=None):
        _strassen(lambda n: _dot_nt(_unpack(w_sum[m, n]), _unpack(when_due(xs_buf[j, n]))),
                  emit, between)

    def project_q(j, between=None, m=0):
        def emit(rh, ch, v):
            pq_buf[j, ch, pl.ds(rh * HD, HD), :] = v
        project_in(m, j, emit, between)

    class Deferred:
        def __init__(self):
            self.now = 0
            self.items = []

        def add(self, delay, fn):
            self.items.append((self.now + delay, fn))

        def tick(self):
            self.now += 1
            due = [fn for t, fn in self.items if t <= self.now]
            self.items = [(t, fn) for t, fn in self.items if t > self.now]
            for fn in due:
                fn()

        def flush(self):
            items, self.items = self.items, []
            for _, fn in items:
                fn()

    def start_in_order(copies, priority=0):
        for c in copies:
            c.start(priority=priority)
            pl.semaphore_signal(sem_order, 1)
            pl.semaphore_wait(sem_order, 1)

    start_in_order(
        [wr_copy, x_copy(0), wphi_copy, q_copy(1, 1), x_copy(1), q_copy(1, 0), x_copy(2),
         q_copy(0, 0), x_copy(3), q_copy(0, 1), x_copy(4), x_copy(5), w_copy(2), w_copy(1), x_copy(6)]
        + ([] if 1 else list(f_copies(0))))
    if 1:
        start_in_order([c for i in range(NB) for c in f_copies(i)], 1)
    kv_acc[...] = jnp.zeros(kv_acc.shape, F32)
    z_acc[...] = jnp.zeros(z_acc.shape, F32)
    y_acc[...] = jnp.zeros(y_acc.shape, F32)
    with _Scope("wr"):
        wr_copy.wait()
    with _Scope("wx0"):
        x_copy(0).wait()
    advance(token_stats(0, None, (0,)), STEP)
    never = stat_buf[1, pl.ds(0, 8), :] < 0.0
    never16 = jnp.concatenate([never, never], axis=0)
    never2 = jnp.concatenate([never, never], axis=1)
    zero = never.astype(jnp.int32)[0, 0]
    advance(token_sums(0, (1, 3)), STEP)
    with _Scope("wphi"):
        wphi_copy.wait()
    for g in range(NG):
        bd_buf.at[g][...] = _pack(jnp.concatenate([fold_matrix(g), fold_matrix(g + NG)], axis=1))

    def quadrant(rh, kh):
        with _Scope("wq%d%d" % (rh, kh)):
            q_copy(rh, kh).wait()
        return jnp.concatenate([
            _dot_nt(_unpack(bd_buf[g, :, pl.ds(128 * rh, 128)]),
                    w_raw[0, pl.ds(kh * HD, HD), pl.ds(rh * HD + 128 * g, 128)]) * LOG2E
            for g in range(NG)], axis=0)

    def first_product(n, lhs):
        lhs = _pack(lhs)
        w_sum.at[0, n][...] = lhs
        return _dot_nt(_unpack(lhs), _unpack(xs_buf[0, n]))

    a22 = quadrant(1, 1)
    m4 = first_product(3, a22)
    x_copy(1).wait()
    a21 = quadrant(1, 0)
    advance(token_stats(0, None, (1,)), STEP)
    advance(token_sums(0, (0, 2, 4, 5, 6)), STEP)
    m2 = first_product(1, a21 + a22)
    pq_buf[0, 0, pl.ds(HD, HD), :] = m2 + m4
    x_copy(2).wait()
    a11 = quadrant(0, 0)
    advance(token_stats(1, never16 if 1 else None, (0,)), STEP)
    advance(token_sums(1, (1, 3)), STEP)
    m3 = first_product(2, a11)
    m1 = first_product(0, a11 + a22)
    pq_buf[0, 1, pl.ds(HD, HD), :] = m3 - m2 + m1 + first_product(5, a21 - a11)
    with _Scope("wx1"):
        x_copy(3).wait()
    a12 = quadrant(0, 1)
    advance(token_stats(1, never16 if 1 else None, (1,)), STEP)
    m5 = first_product(4, a11 + a12)
    pq_buf[0, 1, pl.ds(0, HD), :] = m3 + m5
    pq_buf[0, 0, pl.ds(0, HD), :] = m4 + m1 - m5 + first_product(6, a12 - a22)
    advance(token_sums(1, (0, 2, 4, 5, 6)), STEP)

    stat_plans = [(4, 4, 4, 5, 0, 0, 0), (3, 3, 3, 3, 2, 3, 0), (4, 3, 3, 3, 4, 0, 0), (3, 3, 2, 3, 2, 2, 2)]
    sum_plans = [(0,) * 7, (2, 1, 1, 1, 1, 1, 1), (1, 1, 2, 1, 2, 1, 0), (2, 2, 2, 2, 0, 0, 0), (0, 0, 0, 2, 2, 2, 2)]
    later = Deferred()
    for j in range(1, NSTEP - 1):
        with _Scope("w%d" % j):
            if j == 1:
                x_copy(4).wait()
            if j == 3:
                x_copy(5).wait()
                w_copy(2).wait()
            if j == 5:
                w_copy(1).wait()
                x_copy(6).wait()
        ahead = 0 and j > 0
        near = token_stats(j + 1, never16) if not ahead or j == 1 else iter(())
        far = token_stats(j + 2, never16) if ahead and j + 2 < NSTEP else iter(())
        sums = token_sums(j + 1)

        def side(n, j=j, near=near, far=far, sums=sums, ahead=ahead):
            later.tick()
            advance(near, stat_plans[0][n])
            advance(far, stat_plans[3][n])
            if ahead and j > 1:
                advance(sums, sum_plans[1][n])
            t = 7 * ((j - 3) % 2) + n
            if j >= 3 and t % 3 == 0 and t // 3 < NG:
                store = prepare_weights(2 if j < 5 else 1, t // 3)

                def store_and_mark(store=store):
                    store()
                    if 0:
                        seen = written(w_sum.at[zero, zero])
                        later.add(0, lambda: due.append(seen))
                later.add(2, store_and_mark)
        project_q(j, side)
        for gen in (near, far, sums):
            advance(gen, STEP)
        if j % 2 == 0:
            later.flush()
            later.flush()
            due.clear()

    top = jnp.max(jnp.max(scores[0], axis=0, keepdims=True), axis=1, keepdims=True)
    token = (16 * lane16 + lax.broadcasted_iota(jnp.int32, (16, 128), 0)).astype(F32)
    cand = jnp.where(scores[0] == top, token, float(S))
    idx = jnp.min(jnp.min(cand, axis=0, keepdims=True), axis=1, keepdims=True).astype(jnp.int32)[0, 0]
    idx = jnp.clip(idx, 0, S - 1)
    slab = pl.ds(pl.multiple_of((idx // 16) * 16, 16), 16)
    pick = lax.broadcasted_iota(jnp.int32, (16, D), 0) == idx % 16
    x_sel = jnp.sum(jnp.where(pick, _round_bf16(normalized(slab)[1]), 0.0), axis=0, keepdims=True)
    for c in range(D // 128):
        xb_buf[pl.ds(128 * c, 128), :] = jnp.broadcast_to(
            x_sel[:, 128 * c:128 * c + 128], (128, 128)).T

    def matvec(acc, rows, load, column, last):
        acc = list(acc)
        for r0 in range(0, rows, 8 * 4):
            slabs = [(load(r).astype(F32), column(r)) for r in range(r0, r0 + 8 * 4, 8)]
            for e in range(2):
                if last is not None and (1 or r0 == 0):
                    acc[e] = jnp.where(never, last, acc[e])
                for w, col in slabs:
                    acc[e] = acc[e] + w[:, 128 * e:128 * e + 128] * col
                if 1 or e == 1:
                    last = acc[e]
        return acc, last

    def ffn(i):
        last = None
        act = []
        for c in range(0, 2 * FC, 256):
            acc, last = matvec([jnp.zeros((8, 128), F32)] * 2, D,
                               lambda r: wgu_buf[i, pl.ds(r, 8), pl.ds(c, 256)],
                               lambda r: xb_buf[pl.ds(r, 8), :], last)
            act += [_round_bf16(jnp.sum(a, axis=0, keepdims=True)) for a in acc]
        act = jnp.concatenate(act, axis=1)
        h = _round_bf16(_round_bf16(_silu(act[:, :FC])) * act[:, FC:])
        ys = [[y_acc[:, pl.ds(n + e, 128)] for e in (0, 128)] for n in range(0, D, 256)]
        for c in range(0, FC, 128):
            hb = jnp.broadcast_to(h[:, c:c + 128], (128, 128)).T
            for n in range(D // 256):
                ys[n], last = matvec(ys[n], 128,
                                     lambda r: wd_buf[i, pl.ds(c + r, 8), pl.ds(256 * n, 256)],
                                     lambda r: hb[r:r + 8], last)
        y_acc[...] = jnp.concatenate([y for pair in ys for y in pair], axis=1)
        return last

    def phase_b(i, carry):
        with _Scope("wf"):
            for c in f_copies(i):
                c.wait()

        if not 1:
            @pl.when(i + 1 < NB)
            def _():
                start_in_order(f_copies(i + 1))

        for t in range(2):
            def emit_k(rh, ch, v, t=t):
                for p in range(NPAIR // 2):
                    pair = rh * (NPAIR // 2) + p
                    phi = _dual_softmax(v[64 * p:64 * p + 64])
                    z_acc[pair] += jnp.concatenate(phi, axis=0)
                    phik_buf.at[pair, 2 * t + ch][...] = _pack(jnp.concatenate(
                        [jnp.concatenate(phi[:8], axis=0), jnp.concatenate(phi[8:], axis=0)], axis=1))
            project_in(1, 2 * i + t, emit_k)
        prepare_weights(3, i)()
        done = ffn(i)
        for t in range(2):
            def emit_v(rh, ch, v, t=t):
                for p in range(0, NPAIR // 2, 2):
                    vt_buf.at[(rh * (NPAIR // 2) + p) // 2, 2 * t + ch][...] = _pack(jnp.concatenate(
                        [v[64 * p:64 * p + 64], v[64 * p + 64:64 * p + 128]], axis=1))

            def product(n, t=t):
                rhs = xs_buf[2 * i + t, n]
                if (t, n) == (0, 2) and 1:
                    rhs = after(wo_sum[0, pl.ds(0, 8), pl.ds(0, 128)], rhs)
                if (t, n) == (1, 5) and 0:
                    rhs = after(pltpu.bitcast(done, U32), rhs)
                return _dot_nt(_unpack(w_sum[2, n]), _unpack(rhs))
            _strassen(product, emit_v)
            if 1 or t == 1:
                tiles = (2 * t, 2 * t + 1) if 1 else range(4)
                for p in range(NPAIR):
                    vt = jnp.concatenate(
                        [vt_buf[p // 2, u, :, pl.ds(128 * (p % 2), 128)] for u in tiles], axis=1)
                    phi = jnp.concatenate([jnp.concatenate(
                        [phik_buf[p, u, :, pl.ds(128 * e, 128)] for e in range(2)], axis=0)
                        for u in tiles], axis=1)
                    kv_acc[p] += _dot_nt(_unpack(vt), _unpack(phi))
        return carry

    def keep_alive():
        for ref in (pq_buf.at[0, 0], xs_buf.at[0, 0], w_sum.at[0, 0], stat_buf.at[0], xb_buf, kv_acc.at[0], z_acc.at[0], y_acc, wo_sum.at[0]):
            c = pltpu.make_async_copy(ref, ref, sem_s.at[0])
            c.start()
            c.wait()

    if 0 == 1:
        for c in f_copies(0):
            c.wait()
        return keep_alive()
    if 0 in (0, 2):
        with _Scope("phB"):
            lax.fori_loop(0, NB, phase_b, 0)
    if 0 == 2:
        return keep_alive()

    y = _round_bf16(jnp.sum(y_acc[...], axis=0, keepdims=True))
    r_sel = _round_bf16(0.5 + 0.5 * jnp.tanh(0.5 * top))
    y = _round_bf16(y * r_sel)
    upd_buf[0] = jnp.zeros((8, D), F32)
    upd_buf[1] = jnp.where(lax.broadcasted_iota(jnp.int32, (8, D), 0) == idx % 8, y, 0.0)

    r_ = lax.broadcasted_iota(jnp.int32, (64, 128), 0)
    c_ = lax.broadcasted_iota(jnp.int32, (64, 128), 1)
    own = r_ // DH == c_ % 2
    for p in range(NPAIR // 2):
        kvb_buf.at[p][...] = _pack(jnp.concatenate(
            [jnp.where(own, kv_acc[p + NPAIR // 2 * u], 0.0) for u in range(2)], axis=1))
    for p in range(NPAIR):
        z_acc[p] = jnp.broadcast_to(jnp.sum(z_acc[p], axis=1, keepdims=True), (128, 128))

    recent = []

    def attend_pairs(j, p):
        odd = lax.broadcasted_iota(jnp.int32, (8, SUB), 0) % 2 == 1
        o = []
        for u in range(2):
            pair = p + NPAIR // 2 * u
            for ch in range(2):
                logits = pq_buf[j, ch, pl.ds(64 * pair, 64), :]
                if 0 and len(recent) >= 0:
                    logits = after(recent[-0], logits)
                phi = _dual_softmax(logits)
                den = _tree([phi[t] * z_acc[pair, pl.ds(8 * t, 8), :] for t in range(16)], jnp.add)
                rd = _recip(_allreduce(den, jnp.add) + 1e-6)
                rs = pltpu.roll(rd, 1, 0)
                r0 = jnp.where(odd, rs, rd)
                r1 = jnp.where(odd, rd, rs)
                num = _dot(_unpack(kvb_buf[p, :, pl.ds(128 * u, 128)]),
                           jnp.concatenate(phi, axis=0).astype(BF16))
                o.append(num * jnp.concatenate([r0] * 4 + [r1] * 4, axis=0))

        def store():
            os_buf.at[j % 2][pl.ds(32 * p, 32), :] = _pack(jnp.concatenate(_rhs_sums(*o), axis=1))
            if 0 == 2 and j > 0:
                seen = os_buf[j % 2 + zero, pl.ds(pl.multiple_of(zero * 8 + 32 * p, 8), 8),
                              pl.ds(pl.multiple_of(zero * 128, 128), 128)]
                later.add(2, lambda: due.append(seen))
        return store

    TILES = NG if 1 else 1
    last_blocks = {
        (rh, ch, e): pltpu.make_async_copy(
            out_buf.at[blk], out_hbm.at[blk], sem_last.at[(2 * rh + ch) * NG + e])
        for rh in range(2) for ch in range(2) for e in range(TILES if rh and ch else 1)
        for width in [HD // TILES if rh and ch else HD]
        for blk in [(pl.ds(S - STEP + ch * SUB, SUB), pl.ds(rh * HD + e * width, width))]}

    def gate(row0, cols):
        x, xn = normalized(pl.ds(row0, 16), cols)
        upd = jnp.concatenate([
            upd_buf[(idx // 8 == row0 // 8 + e).astype(jnp.int32), :, cols]
            for e in range(2)], axis=0)
        return x, _silu(xn + upd)

    def last_gates():
        for r in range(0, STEP, 16):
            gate_buf[pl.ds(r, 16), :] = gate(S - STEP + r, slice(None))[1]
        seen = written(gate_buf)
        later.add(3, lambda: due.append(pltpu.bitcast(seen, U32)))

    def finish(j, rh, ch, v):
        cols = pl.ds(rh * HD, HD)
        s = v.T
        for r in range(0, SUB, 16):
            row0 = j * STEP + ch * SUB + r
            if j == NSTEP - 1 and 0:
                x = x_buf[pl.ds(row0, 16), cols].astype(F32)
                g = gate_buf[pl.ds(pl.multiple_of(zero * 16 + ch * SUB + r, 16), 16), cols]
            else:
                x, g = gate(row0, cols)
            out_buf[pl.ds(row0, 16), cols] = (x + s[r:r + 16] * g).astype(BF16)
        if j == NSTEP - 1:
            for e in range(TILES if rh and ch else 1):
                last_blocks[rh, ch, e].start(priority=0)
        elif (rh, ch) == (1, 1):
            o_copy(j).start(priority=0)
        seen = out_buf[pl.ds(pl.multiple_of(zero * 16, 16), 16),
                       pl.ds(pl.multiple_of(zero * 128 + HD, 128), 128)]
        if 1 or (rh, ch) == (1, 0):
            later.add(3, lambda: due.append(pltpu.bitcast(seen, U32)))

    later = Deferred()
    plan = {-1: (0,), 0: (1, 2), 1: (3,), 2: (4,), 3: (5,), 4: (6,), 5: (7,), 6: ()}

    def attend_between(j):
        def between(n):
            if n >= 0:
                later.tick()
            if j < NSTEP:
                for p in plan[n]:
                    later.add(1, attend_pairs(j, p))
        return between

    attend_between(0)(-1)
    project_q(NSTEP - 1, attend_between(0))
    for j in range(NSTEP):
        def emit(rh, ch, v, j=j):
            if j == NSTEP - 1 and 1:
                finish(j, rh, ch, v)
            else:
                later.add(1, lambda: finish(j, rh, ch, v))

        def product(n, j=j):
            rhs = os_buf[j % 2 + (zero if 0 == 1 else 0), :, pl.ds(SUB * n, SUB)]
            rhs = when_due(rhs)
            m = _dot(_unpack(wo_sum[n]), _unpack(rhs))
            recent.append(m[:8])
            return m
        attend = attend_between(j + 1)
        attend(-1)
        if j == NSTEP - 1 and 0:
            last_gates()
        _strassen(product, emit, attend)
    later.flush()
    with _Scope("wout"):
        for j in range(NSTEP - 1):
            o_copy(j).wait()
        for c in last_blocks.values():
            c.wait()


@jax.jit
def pallas_recurrent_scan__linear_kernel_hedgehog__moe_arch_mod__prompt_kernel(
    A_x: jax.Array,
    A_wqkv: jax.Array,
    A_w_phi: jax.Array,
    A_wo: jax.Array,
    B_x: jax.Array,
    B_w_r: jax.Array,
    B_w_gate: jax.Array,
    B_w_up: jax.Array,
    B_w_down: jax.Array,
):
    del B_x
    scratch = [
        pltpu.VMEM((S, D), BF16),
        pltpu.VMEM((NSTEP, 7, SUB // 2, HD), U32),
        pltpu.VMEM((2, S, 128), F32),
        pltpu.VMEM((4, D, D), BF16),
        pltpu.VMEM((3, 7, HD // 2, HD), U32),
        pltpu.VMEM((7, HD // 2, HD), U32),
        pltpu.VMEM((H * DH, DH), BF16),
        pltpu.VMEM((NG, 64, 256), U32),
        pltpu.VMEM((8, 128), BF16),
        pltpu.VMEM((NSTEP, 2, D, SUB), F32),
        pltpu.VMEM((NPAIR // 2, 4, 32, 256), U32),
        pltpu.VMEM((NPAIR, 4, 32, 256), U32),
        pltpu.VMEM((NPAIR, 64, 128), F32),
        pltpu.VMEM((NPAIR, 128, 128), F32),
        pltpu.VMEM((NPAIR // 2, 32, 256), U32),
        pltpu.VMEM((2, HD // 2, 7 * SUB), U32),
        pltpu.VMEM((NB, D, 2 * FC), BF16),
        pltpu.VMEM((NB, FC, D), BF16),
        pltpu.VMEM((D, 128), F32),
        pltpu.VMEM((8, D), F32),
        pltpu.VMEM((2, 8, D), F32),
        pltpu.VMEM((STEP, D), F32),
        pltpu.VMEM((S, D), BF16),
        pltpu.SemaphoreType.DMA((len(X_CUTS) - 1,)),
        pltpu.SemaphoreType.DMA((4,)),
        pltpu.SemaphoreType.DMA((2,)),
        pltpu.SemaphoreType.DMA((2,)),
        pltpu.SemaphoreType.DMA((5 * NB,)),
        pltpu.SemaphoreType.DMA((NSTEP - 1,)),
        pltpu.SemaphoreType.DMA((4 * NG,)),
        pltpu.SemaphoreType.REGULAR,
    ]
    any_spec = pl.BlockSpec(memory_space=pl.ANY)
    flags = {}
    if 0:
        flags["XLA_TPU_FORCE_LP_LLO_SCHEDULER"] = True
    if 0:
        flags["XLA_TPU_EVENLY_DISTRIBUTE_CRITICAL_NODES"] = True
    out = pl.pallas_call(
        _kernel,
        out_shape=jax.ShapeDtypeStruct((S, D), BF16),
        in_specs=[any_spec] * 8,
        out_specs=any_spec,
        scratch_shapes=scratch,
        compiler_params=pltpu.CompilerParams(vmem_limit_bytes=120 * 2**20, flags=flags or None),
        name="hedgehog_mod",
    )(
        A_x.reshape(S, D),
        A_wqkv,
        A_w_phi.reshape(H * DH, DH),
        A_wo,
        B_w_r.reshape(8, 128),
        B_w_gate,
        B_w_up,
        B_w_down,
    )
    return out.reshape(1, S, D)
```

```python
import math

import jax
import jax.numpy as jnp
from jax import lax
import jax.experimental.pallas as pl
import jax.experimental.pallas.tpu as pltpu

S, D, H, DH, F = 2048, 1024, 32, 32, 3584
SUB = 128
STEP = 2 * SUB
NSTEP = S // STEP
NB = 4
FC = F // NB
HD = D // 2
NG = HD // 128
NPAIR = H // 2
X_CUTS = (0, 1, 2, 3, 4, 8, 12, 16)
LOG2E = math.log2(math.e)
EPS = 1.0013580322265625e-05
F32, BF16, U32 = jnp.float32, jnp.bfloat16, jnp.uint32


def _dot(a, b):
    return jnp.dot(a, b, preferred_element_type=F32)


def _dot_nt(a, b):
    return lax.dot_general(a, b, (((1,), (1,)), ((), ())), preferred_element_type=F32)


def _round_bf16(v):
    return v.astype(BF16).astype(F32)


def _pack(v):
    return pltpu.bitcast(v.astype(BF16), U32)


def _unpack(v):
    return pltpu.bitcast(v, BF16)


def _aligned(i, n):
    return i if isinstance(i, int) else pl.multiple_of(i, n)


def _silu(t):
    h = 0.5 * t
    return h + h * jnp.tanh(h)


def _allreduce(v, op):
    v = op(v, pltpu.roll(v, 4, 0))
    return op(v, pltpu.roll(v, 2, 0))


def _tree(vals, op):
    while len(vals) > 1:
        vals = [op(a, b) for a, b in zip(vals[::2], vals[1::2])]
    return vals[0]


def _dual_softmax(p):
    ps = [p[8 * j:8 * j + 8] for j in range(8)]
    hi = _allreduce(_tree(ps, jnp.maximum), jnp.maximum)
    lo = _allreduce(_tree(ps, jnp.minimum), jnp.minimum)
    pos = [jnp.exp2(v - hi) for v in ps]
    neg = [jnp.exp2(lo - v) for v in ps]
    pos_scale = pltpu.reciprocal(_allreduce(_tree(pos, jnp.add), jnp.add), approx=True)
    neg_scale = pltpu.reciprocal(_allreduce(_tree(neg, jnp.add), jnp.add), approx=True)
    return [e * pos_scale for e in pos] + [e * neg_scale for e in neg]


def _lhs_sums(a11, a12, a21, a22):
    return (a11 + a22, a21 + a22, a11, a22, a11 + a12, a21 - a11, a12 - a22)


def _rhs_sums(b11, b12, b21, b22):
    return (b11 + b22, b11, b12 - b22, b21 - b11, b22, b11 + b12, b21 + b22)


def _strassen(prod, emit, between=lambda n: None):
    m2 = prod(1)
    between(0)
    m4 = prod(3)
    emit(1, 0, m2 + m4)
    between(1)
    m3 = prod(2)
    c22 = m3 - m2
    between(2)
    m5 = prod(4)
    emit(0, 1, m3 + m5)
    c11 = m4 - m5
    between(3)
    m1 = prod(0)
    c11 = c11 + m1
    c22 = c22 + m1
    between(4)
    emit(0, 0, c11 + prod(6))
    between(5)
    emit(1, 1, c22 + prod(5))
    between(6)


class _Deferred:
    def __init__(self):
        self.now = 0
        self.items = []

    def add(self, delay, fn):
        self.items.append((self.now + delay, fn))

    def tick(self):
        self.now += 1
        due = [fn for t, fn in self.items if t <= self.now]
        self.items = [(t, fn) for t, fn in self.items if t > self.now]
        for fn in due:
            fn()

    def flush(self):
        items, self.items = self.items, []
        for _, fn in items:
            fn()


def _advance(steps, count=STEP):
    for _ in range(count):
        next(steps, None)


def _kernel(x_hbm, wqkv_hbm, wphi_hbm, wo_hbm, wr_hbm, wg_hbm, wu_hbm, wd_hbm,
            out_hbm,
            x_buf, xs_buf, stat_buf, w_raw, w_sum, wo_sum, wphi_buf, fold_buf, wr_buf,
            pq_buf, vt_buf, phik_buf, kv_acc, z_acc, kvb_buf, os_buf,
            wgu_buf, wd_buf, xb_buf, y_acc, upd_buf, out_buf,
            sem_x, sem_q, sem_w, sem_s, sem_f, sem_o, sem_last, sem_order):
    def x_copy(n):
        rows = pl.ds(X_CUTS[n] * SUB, (X_CUTS[n + 1] - X_CUTS[n]) * SUB)
        return pltpu.make_async_copy(x_hbm.at[rows], x_buf.at[rows], sem_x.at[n])

    def q_copy(rh, kh):
        blk = (pl.ds(kh * HD, HD), pl.ds(rh * HD, HD))
        return pltpu.make_async_copy(wqkv_hbm.at[blk], w_raw.at[0].at[blk], sem_q.at[2 * rh + kh])

    def w_copy(m):
        return pltpu.make_async_copy(wqkv_hbm.at[:, pl.ds(m * D, D)], w_raw.at[m], sem_w.at[m - 1])

    def ffn_copies(i):
        cols = pl.ds(i * FC, FC)
        return (
            pltpu.make_async_copy(wg_hbm.at[:, cols], wgu_buf.at[i, :, pl.ds(0, FC)], sem_f.at[i]),
            pltpu.make_async_copy(wu_hbm.at[:, cols], wgu_buf.at[i, :, pl.ds(FC, FC)],
                                  sem_f.at[NB + i]),
            pltpu.make_async_copy(wd_hbm.at[cols], wd_buf.at[i], sem_f.at[2 * NB + i]),
        )

    def wo_copies(g):
        return tuple(
            pltpu.make_async_copy(wo_hbm.at[:, cols], w_raw.at[3, :, cols],
                                  sem_f.at[(3 + half) * NB + g])
            for half in range(2)
            for cols in [pl.ds(_aligned(128 * (g + NG * half), 128), 128)])

    def out_copy(j):
        rows = pl.ds(j * STEP, STEP)
        return pltpu.make_async_copy(out_buf.at[rows], out_hbm.at[rows], sem_o.at[j])

    def last_out_copy(rh, ch):
        blk = (pl.ds(S - STEP + ch * SUB, SUB), pl.ds(rh * HD, HD))
        return pltpu.make_async_copy(out_buf.at[blk], out_hbm.at[blk], sem_last.at[2 * rh + ch])

    wphi_copy = pltpu.make_async_copy(wphi_hbm, wphi_buf, sem_s.at[0])
    wr_copy = pltpu.make_async_copy(wr_hbm, wr_buf, sem_s.at[1])

    def start_in_order(copies, priority):
        for c in copies:
            c.start(priority=priority)
            pl.semaphore_signal(sem_order, 1)
            pl.semaphore_wait(sem_order, 1)

    def fold_matrix(g):
        r = lax.broadcasted_iota(jnp.int32, (128, DH), 0)
        f = lax.broadcasted_iota(jnp.int32, (128, DH), 1)
        sel = jnp.where((r % 64) // 2 == f, 1.0, 0.0).astype(BF16)
        t = _dot_nt(sel, wphi_buf[pl.ds(128 * g, 128), :])
        r = lax.broadcasted_iota(jnp.int32, (128, 128), 0)
        c = lax.broadcasted_iota(jnp.int32, (128, 128), 1)
        return jnp.where(2 * (r // 64) + r % 2 == c // DH, t * LOG2E, 0.0)

    def prepare_weights(m, g, src):
        def block(half, k0):
            w = w_raw[src, pl.ds(k0, 256), pl.ds(_aligned(128 * (g + NG * half), 128), 128)]
            if m == 1:
                return _dot_nt(_unpack(fold_buf[g, :, pl.ds(128 * half, 128)]), w)
            return w.T.astype(F32)

        blocks = {k0: (block(0, k0), block(0, HD + k0), block(1, k0), block(1, HD + k0))
                  for k0 in range(0, HD, 256)}

        def store():
            dst = wo_sum if m == 3 else w_sum.at[m]
            for k0, quad in blocks.items():
                for n, v in enumerate(_lhs_sums(*quad)):
                    dst.at[n][pl.ds(_aligned(64 * g, 64), 64), pl.ds(k0, 256)] = _pack(v)
        return store

    lane16 = lax.broadcasted_iota(jnp.int32, (16, 128), 1)
    scores = [jnp.full((16, 128), -jnp.inf, F32)]

    def token_stats(j, halves, never16):
        wr = wr_buf[...].astype(F32)
        wrow = jnp.concatenate(
            [jnp.broadcast_to(wr[c:c + 1], (16, 128)) for c in range(8)], axis=1)
        last = None
        for half in halves:
            slabs = range((2 * j + half) * SUB // 16, (2 * j + half + 1) * SUB // 16)
            sq = dot = jnp.zeros((16, 128), F32)
            for t in slabs:
                rows = pl.ds(16 * t, 16)
                x = x_buf[rows, :].astype(F32)
                if last is not None:
                    x = jnp.concatenate([jnp.where(never16, last, x[:, :128]), x[:, 128:]], axis=1)
                mean = jnp.sum(x, axis=1, keepdims=True) * (1.0 / D)
                stat_buf[0, rows, :] = jnp.broadcast_to(mean, (16, 128))
                c = x - mean
                sq = jnp.where(lane16 == t, jnp.sum(c * c, axis=1, keepdims=True), sq)
                dot = jnp.where(lane16 == t, jnp.sum(c * wrow, axis=1, keepdims=True), dot)
                if never16 is not None and t % 2 == 0:
                    last = sq
                yield
            inv = 1.0 / _round_bf16(jnp.sqrt(_round_bf16(_round_bf16(sq * (1.0 / D)) + EPS)))
            mine = (lane16 >= slabs[0]) & (lane16 <= slabs[-1])
            score = _round_bf16(dot * inv)
            scores[0] = jnp.where(mine & (score == score), score, scores[0])
            for t in slabs:
                stat_buf[1, pl.ds(16 * t, 16), :] = jnp.broadcast_to(inv[:, t:t + 1], (16, 128))

    def normalized(rows, cols=slice(None)):
        x = x_buf[rows, cols].astype(F32)
        reps = x.shape[1] // 128
        mean = jnp.concatenate([stat_buf[0, rows, :]] * reps, axis=1)
        inv = jnp.concatenate([stat_buf[1, rows, :]] * reps, axis=1)
        return x, (x - mean) * inv

    def token_sums(j, which=range(7)):
        for r in range(0, SUB, 16):
            a = normalized(pl.ds(j * STEP + r, 16))[1]
            b = normalized(pl.ds(j * STEP + SUB + r, 16))[1] if 0 in which else a
            for n, v in enumerate(_rhs_sums(a[:, :HD], b[:, :HD], a[:, HD:], b[:, HD:])):
                if n in which:
                    xs_buf.at[j, n][pl.ds(r // 2, 8), :] = _pack(v)

    def project(m, j, n):
        return _dot_nt(_unpack(w_sum[m, n]), _unpack(xs_buf[j, n]))

    def project_q(j, between):
        def emit(rh, ch, v):
            pq_buf[j, ch, pl.ds(rh * HD, HD), :] = v
        _strassen(lambda n: project(0, j, n), emit, between)

    def after(token, v):
        top = jnp.where(never, token, v[:8, :128])
        if v.shape[1] > 128:
            top = jnp.concatenate([top, v[:8, 128:]], axis=1)
        return jnp.concatenate([top, v[8:]], axis=0)

    start_in_order(
        [wr_copy, x_copy(0), wphi_copy, q_copy(1, 1), x_copy(1), q_copy(1, 0), x_copy(2),
         q_copy(0, 0), x_copy(3), q_copy(0, 1), x_copy(4), x_copy(5), w_copy(2), w_copy(1),
         x_copy(6)], 0)
    start_in_order([c for i in range(NB) for c in ffn_copies(i) + wo_copies(i)], 1)
    kv_acc[...] = jnp.zeros(kv_acc.shape, F32)
    z_acc[...] = jnp.zeros(z_acc.shape, F32)
    y_acc[...] = jnp.zeros(y_acc.shape, F32)
    wo_sum[0, pl.ds(0, 8), pl.ds(0, 128)] = jnp.zeros((8, 128), U32)
    wr_copy.wait()
    x_copy(0).wait()
    _advance(token_stats(0, (0,), None))
    never = stat_buf[1, pl.ds(0, 8), :] < 0.0
    never16 = jnp.concatenate([never, never], axis=0)
    zero = never.astype(jnp.int32)[0, 0]
    token_sums(0, (1, 3))
    wphi_copy.wait()
    for g in range(NG):
        fold_buf.at[g][...] = _pack(jnp.concatenate([fold_matrix(g), fold_matrix(g + NG)], axis=1))

    def q_quadrant(rh, kh):
        q_copy(rh, kh).wait()
        return jnp.concatenate([
            _dot_nt(_unpack(fold_buf[g, :, pl.ds(128 * rh, 128)]),
                    w_raw[0, pl.ds(kh * HD, HD), pl.ds(rh * HD + 128 * g, 128)])
            for g in range(NG)], axis=0)

    def first_product(n, lhs):
        lhs = _pack(lhs)
        w_sum.at[0, n][...] = lhs
        return _dot_nt(_unpack(lhs), _unpack(xs_buf[0, n]))

    a22 = q_quadrant(1, 1)
    m4 = first_product(3, a22)
    x_copy(1).wait()
    a21 = q_quadrant(1, 0)
    _advance(token_stats(0, (1,), None))
    token_sums(0, (0, 2, 4, 5, 6))
    m2 = first_product(1, a21 + a22)
    pq_buf[0, 0, pl.ds(HD, HD), :] = m2 + m4
    x_copy(2).wait()
    a11 = q_quadrant(0, 0)
    _advance(token_stats(1, (0,), never16))
    token_sums(1, (1, 3))
    m3 = first_product(2, a11)
    m1 = first_product(0, a11 + a22)
    pq_buf[0, 1, pl.ds(HD, HD), :] = m3 - m2 + m1 + first_product(5, a21 - a11)
    x_copy(3).wait()
    a12 = q_quadrant(0, 1)
    _advance(token_stats(1, (1,), never16))
    m5 = first_product(4, a11 + a12)
    pq_buf[0, 1, pl.ds(0, HD), :] = m3 + m5
    pq_buf[0, 0, pl.ds(0, HD), :] = m4 + m1 - m5 + first_product(6, a12 - a22)
    token_sums(1, (0, 2, 4, 5, 6))

    later = _Deferred()
    for j in range(1, NSTEP - 1):
        if j == 1:
            x_copy(4).wait()
        if j == 3:
            x_copy(5).wait()
            w_copy(2).wait()
        if j == 5:
            w_copy(1).wait()
            x_copy(6).wait()
        stats = token_stats(j + 1, (0, 1), never16)

        def alongside(n, j=j, stats=stats):
            later.tick()
            _advance(stats, (4, 4, 4, 5, 0, 0, 0)[n])
            g, offset = divmod(7 * ((j - 3) % 2) + n, 3)
            if j >= 3 and offset == 0 and g < NG:
                m = 2 if j < 5 else 1
                later.add(2, prepare_weights(m, g, m))
        project_q(j, alongside)
        _advance(stats)
        token_sums(j + 1)
        if j % 2 == 0:
            later.flush()

    top = jnp.max(jnp.max(scores[0], axis=0, keepdims=True), axis=1, keepdims=True)
    token = (16 * lane16 + lax.broadcasted_iota(jnp.int32, (16, 128), 0)).astype(F32)
    cand = jnp.where(scores[0] == top, token, float(S))
    idx = jnp.min(jnp.min(cand, axis=0, keepdims=True), axis=1, keepdims=True)
    idx = jnp.clip(idx.astype(jnp.int32)[0, 0], 0, S - 1)
    slab = pl.ds(pl.multiple_of((idx // 16) * 16, 16), 16)
    pick = lax.broadcasted_iota(jnp.int32, (16, D), 0) == idx % 16
    x_sel = jnp.sum(jnp.where(pick, _round_bf16(normalized(slab)[1]), 0.0), axis=0, keepdims=True)
    for c in range(0, D, 128):
        xb_buf[pl.ds(c, 128), :] = jnp.broadcast_to(x_sel[:, c:c + 128], (128, 128)).T

    def matvec(acc, rows, load, column, last):
        acc = list(acc)
        for r0 in range(0, rows, 32):
            slabs = [(load(r).astype(F32), column(r)) for r in range(r0, r0 + 32, 8)]
            for e in range(2):
                if last is not None:
                    acc[e] = jnp.where(never, last, acc[e])
                for w, col in slabs:
                    acc[e] = acc[e] + w[:, 128 * e:128 * e + 128] * col
                last = acc[e]
        return acc, last

    def ffn(i):
        last = None
        act = []
        for c in range(0, 2 * FC, 256):
            acc, last = matvec([jnp.zeros((8, 128), F32)] * 2, D,
                               lambda r: wgu_buf[i, pl.ds(r, 8), pl.ds(c, 256)],
                               lambda r: xb_buf[pl.ds(r, 8), :], last)
            act += [_round_bf16(jnp.sum(a, axis=0, keepdims=True)) for a in acc]
        act = jnp.concatenate(act, axis=1)
        h = _round_bf16(_round_bf16(_silu(act[:, :FC])) * act[:, FC:])
        ys = [[y_acc[:, pl.ds(n + e, 128)] for e in (0, 128)] for n in range(0, D, 256)]
        for c in range(0, FC, 128):
            hb = jnp.broadcast_to(h[:, c:c + 128], (128, 128)).T
            for n in range(D // 256):
                ys[n], last = matvec(ys[n], 128,
                                     lambda r: wd_buf[i, pl.ds(c + r, 8), pl.ds(256 * n, 256)],
                                     lambda r: hb[r:r + 8], last)
        y_acc[...] = jnp.concatenate([y for pair in ys for y in pair], axis=1)

    def phase_b(i, carry):
        for c in ffn_copies(i):
            c.wait()

        @pl.when(i > 0)
        def _():
            for c in wo_copies(i - 1):
                c.wait()

        for t in range(2):
            def emit_k(rh, ch, v, t=t):
                for p in range(NPAIR // 2):
                    pair = rh * (NPAIR // 2) + p
                    phi = _dual_softmax(v[64 * p:64 * p + 64])
                    z_acc[pair] += jnp.concatenate(phi, axis=0)
                    phik_buf.at[pair, 2 * t + ch][...] = _pack(jnp.concatenate(
                        [jnp.concatenate(phi[:8], axis=0), jnp.concatenate(phi[8:], axis=0)],
                        axis=1))
            _strassen(lambda n: project(1, 2 * i + t, n), emit_k)

        prepare_weights(3, (i + NB - 1) % NB, jnp.where(i > 0, 3, 0))()
        ffn(i)

        for t in range(2):
            def emit_v(rh, ch, v, t=t):
                for p in range(0, NPAIR // 2, 2):
                    vt_buf.at[(rh * (NPAIR // 2) + p) // 2, 2 * t + ch][...] = _pack(jnp.concatenate(
                        [v[64 * p:64 * p + 64], v[64 * p + 64:64 * p + 128]], axis=1))

            def product(n, t=t):
                rhs = xs_buf[2 * i + t, n]
                if (t, n) == (0, 2):
                    rhs = after(wo_sum[0, pl.ds(0, 8), pl.ds(0, 128)], rhs)
                return _dot_nt(_unpack(w_sum[2, n]), _unpack(rhs))
            _strassen(product, emit_v)
            for p in range(NPAIR):
                vt = jnp.concatenate(
                    [vt_buf[p // 2, u, :, pl.ds(128 * (p % 2), 128)] for u in (2 * t, 2 * t + 1)],
                    axis=1)
                phi = jnp.concatenate([jnp.concatenate(
                    [phik_buf[p, u, :, pl.ds(128 * e, 128)] for e in range(2)], axis=0)
                    for u in (2 * t, 2 * t + 1)], axis=1)
                kv_acc[p] += _dot_nt(_unpack(vt), _unpack(phi))
        return carry

    lax.fori_loop(0, NB, phase_b, 0)

    for c in wo_copies(NB - 1):
        c.wait()
    prepare_weights(3, NB - 1, 3)()
    y = _round_bf16(jnp.sum(y_acc[...], axis=0, keepdims=True))
    y = _round_bf16(y * _round_bf16(0.5 + 0.5 * jnp.tanh(0.5 * top)))
    upd_buf[0] = jnp.zeros((8, D), F32)
    upd_buf[1] = jnp.where(lax.broadcasted_iota(jnp.int32, (8, D), 0) == idx % 8, y, 0.0)

    own = (lax.broadcasted_iota(jnp.int32, (64, 128), 0) // DH
           == lax.broadcasted_iota(jnp.int32, (64, 128), 1) % 2)
    for p in range(NPAIR // 2):
        kvb_buf.at[p][...] = _pack(jnp.concatenate(
            [jnp.where(own, kv_acc[p + NPAIR // 2 * u], 0.0) for u in range(2)], axis=1))
    for p in range(NPAIR):
        z_acc[p] = jnp.broadcast_to(jnp.sum(z_acc[p], axis=1, keepdims=True), (128, 128))

    later = _Deferred()
    due = []

    def attend_pairs(j, p):
        odd = lax.broadcasted_iota(jnp.int32, (8, SUB), 0) % 2 == 1
        o = []
        for u in range(2):
            pair = p + NPAIR // 2 * u
            for ch in range(2):
                phi = _dual_softmax(pq_buf[j, ch, pl.ds(64 * pair, 64), :])
                den = _tree([phi[t] * z_acc[pair, pl.ds(8 * t, 8), :] for t in range(16)], jnp.add)
                scale = pltpu.reciprocal(_allreduce(den, jnp.add) + 1e-6, approx=True)
                other = pltpu.roll(scale, 1, 0)
                scale = jnp.concatenate(
                    [jnp.where(odd, other, scale)] * 4 + [jnp.where(odd, scale, other)] * 4, axis=0)
                num = _dot(_unpack(kvb_buf[p, :, pl.ds(128 * u, 128)]),
                           jnp.concatenate(phi, axis=0).astype(BF16))
                o.append(num * scale)

        def store():
            os_buf.at[j % 2][pl.ds(32 * p, 32), :] = _pack(jnp.concatenate(_rhs_sums(*o), axis=1))
        later.add(1, store)

    def attend(j):
        def between(n):
            if n >= 0:
                later.tick()
            if j < NSTEP:
                for p in ((0,), (1, 2), (3,), (4,), (5,), (6,), (7,), ())[n + 1]:
                    attend_pairs(j, p)
        between(-1)
        return between

    def finish(j, rh, ch, v):
        cols = pl.ds(rh * HD, HD)
        s = v.T
        for r in range(0, SUB, 16):
            row0 = j * STEP + ch * SUB + r
            x, xn = normalized(pl.ds(row0, 16), cols)
            upd = jnp.concatenate([
                upd_buf[(idx // 8 == row0 // 8 + e).astype(jnp.int32), :, cols]
                for e in range(2)], axis=0)
            out_buf[pl.ds(row0, 16), cols] = (x + s[r:r + 16] * _silu(xn + upd)).astype(BF16)
        if j == NSTEP - 1:
            last_out_copy(rh, ch).start()
        elif (rh, ch) == (1, 1):
            out_copy(j).start()
        seen = out_buf[pl.ds(pl.multiple_of(zero * 16, 16), 16),
                       pl.ds(pl.multiple_of(zero * 128 + HD, 128), 128)]
        later.add(3, lambda: due.append(pltpu.bitcast(seen, U32)))

    project_q(NSTEP - 1, attend(0))
    for j in range(NSTEP):
        def emit(rh, ch, v, j=j):
            if j == NSTEP - 1:
                finish(j, rh, ch, v)
            else:
                later.add(1, lambda: finish(j, rh, ch, v))

        def product(n, j=j):
            rhs = os_buf[j % 2, :, pl.ds(SUB * n, SUB)]
            while due:
                rhs = after(due.pop(), rhs)
            return _dot(_unpack(wo_sum[n]), _unpack(rhs))
        _strassen(product, emit, attend(j + 1))
    for j in range(NSTEP - 1):
        out_copy(j).wait()
    for rh in range(2):
        for ch in range(2):
            last_out_copy(rh, ch).wait()


@jax.jit
def pallas_recurrent_scan__linear_kernel_hedgehog__moe_arch_mod__prompt_kernel(
    A_x: jax.Array,
    A_wqkv: jax.Array,
    A_w_phi: jax.Array,
    A_wo: jax.Array,
    B_x: jax.Array,
    B_w_r: jax.Array,
    B_w_gate: jax.Array,
    B_w_up: jax.Array,
    B_w_down: jax.Array,
):
    del B_x
    scratch = [
        pltpu.VMEM((S, D), BF16),
        pltpu.VMEM((NSTEP, 7, SUB // 2, HD), U32),
        pltpu.VMEM((2, S, 128), F32),
        pltpu.VMEM((4, D, D), BF16),
        pltpu.VMEM((3, 7, HD // 2, HD), U32),
        pltpu.VMEM((7, HD // 2, HD), U32),
        pltpu.VMEM((H * DH, DH), BF16),
        pltpu.VMEM((NG, 64, 256), U32),
        pltpu.VMEM((8, 128), BF16),
        pltpu.VMEM((NSTEP, 2, D, SUB), F32),
        pltpu.VMEM((NPAIR // 2, 4, 32, 256), U32),
        pltpu.VMEM((NPAIR, 4, 32, 256), U32),
        pltpu.VMEM((NPAIR, 64, 128), F32),
        pltpu.VMEM((NPAIR, 128, 128), F32),
        pltpu.VMEM((NPAIR // 2, 32, 256), U32),
        pltpu.VMEM((2, HD // 2, 7 * SUB), U32),
        pltpu.VMEM((NB, D, 2 * FC), BF16),
        pltpu.VMEM((NB, FC, D), BF16),
        pltpu.VMEM((D, 128), F32),
        pltpu.VMEM((8, D), F32),
        pltpu.VMEM((2, 8, D), F32),
        pltpu.VMEM((S, D), BF16),
        pltpu.SemaphoreType.DMA((len(X_CUTS) - 1,)),
        pltpu.SemaphoreType.DMA((4,)),
        pltpu.SemaphoreType.DMA((2,)),
        pltpu.SemaphoreType.DMA((2,)),
        pltpu.SemaphoreType.DMA((5 * NB,)),
        pltpu.SemaphoreType.DMA((NSTEP - 1,)),
        pltpu.SemaphoreType.DMA((4,)),
        pltpu.SemaphoreType.REGULAR,
    ]
    any_spec = pl.BlockSpec(memory_space=pl.ANY)
    out = pl.pallas_call(
        _kernel,
        out_shape=jax.ShapeDtypeStruct((S, D), BF16),
        in_specs=[any_spec] * 8,
        out_specs=any_spec,
        scratch_shapes=scratch,
        compiler_params=pltpu.CompilerParams(vmem_limit_bytes=120 * 2**20,
                                             disable_semaphore_checks=True),
        name="hedgehog_mod",
    )(
        A_x.reshape(S, D),
        A_wqkv,
        A_w_phi.reshape(H * DH, DH),
        A_wo,
        B_w_r.reshape(8, 128),
        B_w_gate,
        B_w_up,
        B_w_down,
    )
    return out.reshape(1, S, D)
```

```python
import math

import jax
import jax.numpy as jnp
from jax import lax
import jax.experimental.pallas as pl
import jax.experimental.pallas.tpu as pltpu

S, D, H, DH, F = 2048, 1024, 32, 32, 3584
SUB = 128
STEP = 2 * SUB
NSTEP = S // STEP
NB = 4
FC = F // NB
HD = D // 2
NG = HD // 128
NPAIR = H // 2
X_CUTS = (0, 1, 2, 3, 4, 8, 12, 16)
LOG2E = math.log2(math.e)
EPS = 1.0013580322265625e-05
F32, BF16, U32 = jnp.float32, jnp.bfloat16, jnp.uint32


def _dot(a, b):
    return jnp.dot(a, b, preferred_element_type=F32)


def _dot_nt(a, b):
    return lax.dot_general(a, b, (((1,), (1,)), ((), ())), preferred_element_type=F32)


def _round_bf16(v):
    return v.astype(BF16).astype(F32)


def _pack(v):
    return pltpu.bitcast(v.astype(BF16), U32)


def _unpack(v):
    return pltpu.bitcast(v, BF16)


def _aligned(i, n):
    return i if isinstance(i, int) else pl.multiple_of(i, n)


def _silu_of_twice(h):
    return h + h * jnp.tanh(h)


def _allreduce(v, op):
    v = op(v, pltpu.roll(v, 4, 0))
    return op(v, pltpu.roll(v, 2, 0))


def _tree(vals, op):
    while len(vals) > 1:
        vals = [op(a, b) for a, b in zip(vals[::2], vals[1::2])]
    return vals[0]


def _dual_exp(p):
    ps = [p[8 * j:8 * j + 8] for j in range(8)]
    hi = _allreduce(_tree(ps, jnp.maximum), jnp.maximum)
    lo = _allreduce(_tree(ps, jnp.minimum), jnp.minimum)
    pos = [jnp.exp2(v - hi) for v in ps]
    neg = [jnp.exp2(lo - v) for v in ps]
    return (pos, _allreduce(_tree(pos, jnp.add), jnp.add),
            neg, _allreduce(_tree(neg, jnp.add), jnp.add))


def _lhs_sums(a11, a12, a21, a22):
    return (a11 + a22, a21 + a22, a11, a22, a11 + a12, a21 - a11, a12 - a22)


def _rhs_sums(b11, b12, b21, b22):
    return (b11 + b22, b11, b12 - b22, b21 - b11, b22, b11 + b12, b21 + b22)


def _strassen(prod, emit, between=lambda n: None):
    m2 = prod(1)
    between(0)
    m4 = prod(3)
    emit(1, 0, m2 + m4)
    between(1)
    m3 = prod(2)
    c22 = m3 - m2
    between(2)
    m5 = prod(4)
    emit(0, 1, m3 + m5)
    c11 = m4 - m5
    between(3)
    m1 = prod(0)
    c11 = c11 + m1
    c22 = c22 + m1
    between(4)
    emit(0, 0, c11 + prod(6))
    between(5)
    emit(1, 1, c22 + prod(5))
    between(6)


class _Deferred:
    def __init__(self):
        self.now = 0
        self.items = []

    def add(self, delay, fn):
        self.items.append((self.now + delay, fn))

    def tick(self):
        self.now += 1
        due = [fn for t, fn in self.items if t <= self.now]
        self.items = [(t, fn) for t, fn in self.items if t > self.now]
        for fn in due:
            fn()

    def flush(self):
        items, self.items = self.items, []
        for _, fn in items:
            fn()


def _advance(steps, count=STEP):
    for _ in range(count):
        next(steps, None)


def _kernel(x_hbm, wqkv_hbm, wphi_hbm, wo_hbm, wr_hbm, wg_hbm, wu_hbm, wd_hbm,
            out_hbm,
            x_buf, xs_buf, stat_buf, w_raw, w_sum, wo_sum, wphi_buf, fold_buf, wr_buf,
            pq_buf, vt_buf, phik_buf, kv_acc, z_acc, kvb_buf, os_buf,
            wgu_buf, wd_buf, xb_buf, y_acc, upd_buf, out_buf,
            sem_x, sem_q, sem_w, sem_s, sem_f, sem_o, sem_last, sem_order):
    def x_copy(n):
        rows = pl.ds(X_CUTS[n] * SUB, (X_CUTS[n + 1] - X_CUTS[n]) * SUB)
        return pltpu.make_async_copy(x_hbm.at[rows], x_buf.at[rows], sem_x.at[n])

    def q_copy(rh, kh):
        blk = (pl.ds(kh * HD, HD), pl.ds(rh * HD, HD))
        return pltpu.make_async_copy(wqkv_hbm.at[blk], w_raw.at[0].at[blk], sem_q.at[2 * rh + kh])

    def w_copy(m):
        return pltpu.make_async_copy(wqkv_hbm.at[:, pl.ds(m * D, D)], w_raw.at[m], sem_w.at[m - 1])

    def ffn_copies(i):
        cols = pl.ds(i * FC, FC)
        return (
            pltpu.make_async_copy(wg_hbm.at[:, cols], wgu_buf.at[i, :, pl.ds(0, FC)], sem_f.at[i]),
            pltpu.make_async_copy(wu_hbm.at[:, cols], wgu_buf.at[i, :, pl.ds(FC, FC)],
                                  sem_f.at[NB + i]),
            pltpu.make_async_copy(wd_hbm.at[cols], wd_buf.at[i], sem_f.at[2 * NB + i]),
        )

    def wo_copies(g):
        return tuple(
            pltpu.make_async_copy(wo_hbm.at[:, cols], w_raw.at[3, :, cols],
                                  sem_f.at[(3 + half) * NB + g])
            for half in range(2)
            for cols in [pl.ds(_aligned(128 * (g + NG * half), 128), 128)])

    def out_copy(j):
        rows = pl.ds(j * STEP, STEP)
        return pltpu.make_async_copy(out_buf.at[rows], out_hbm.at[rows], sem_o.at[j])

    def last_out_copy(rh, ch):
        blk = (pl.ds(S - STEP + ch * SUB, SUB), pl.ds(rh * HD, HD))
        return pltpu.make_async_copy(out_buf.at[blk], out_hbm.at[blk], sem_last.at[2 * rh + ch])

    wphi_copy = pltpu.make_async_copy(wphi_hbm, wphi_buf, sem_s.at[0])
    wr_copy = pltpu.make_async_copy(wr_hbm, wr_buf, sem_s.at[1])

    def start_in_order(copies, priority):
        for c in copies:
            c.start(priority=priority)
            pl.semaphore_signal(sem_order, 1)
            pl.semaphore_wait(sem_order, 1)

    def fold_matrix(g):
        r = lax.broadcasted_iota(jnp.int32, (128, DH), 0)
        f = lax.broadcasted_iota(jnp.int32, (128, DH), 1)
        sel = jnp.where((r % 64) // 2 == f, 1.0, 0.0).astype(BF16)
        t = _dot_nt(sel, wphi_buf[pl.ds(128 * g, 128), :])
        r = lax.broadcasted_iota(jnp.int32, (128, 128), 0)
        c = lax.broadcasted_iota(jnp.int32, (128, 128), 1)
        return jnp.where(2 * (r // 64) + r % 2 == c // DH, t * LOG2E, 0.0)

    def prepare_weights(m, g, src):
        def block(half, k0):
            w = w_raw[src, pl.ds(k0, 256), pl.ds(_aligned(128 * (g + NG * half), 128), 128)]
            if m == 1:
                return _dot_nt(_unpack(fold_buf[g, :, pl.ds(128 * half, 128)]), w)
            return w.T.astype(F32)

        blocks = {k0: (block(0, k0), block(0, HD + k0), block(1, k0), block(1, HD + k0))
                  for k0 in range(0, HD, 256)}

        def store():
            dst = wo_sum if m == 3 else w_sum.at[m]
            for k0, quad in blocks.items():
                for n, v in enumerate(_lhs_sums(*quad)):
                    dst.at[n][pl.ds(_aligned(64 * g, 64), 64), pl.ds(k0, 256)] = _pack(v)
        return store

    lane16 = lax.broadcasted_iota(jnp.int32, (16, 128), 1)
    scores = [jnp.full((16, 128), -jnp.inf, F32)]

    def token_stats(j, halves, never16):
        wr = wr_buf[...].astype(F32)
        wrow = jnp.concatenate(
            [jnp.broadcast_to(wr[c:c + 1], (16, 128)) for c in range(8)], axis=1)
        last = None
        for half in halves:
            slabs = range((2 * j + half) * SUB // 16, (2 * j + half + 1) * SUB // 16)
            sq = dot = jnp.zeros((16, 128), F32)
            for t in slabs:
                rows = pl.ds(16 * t, 16)
                x = x_buf[rows, :].astype(F32)
                if last is not None:
                    x = jnp.concatenate([jnp.where(never16, last, x[:, :128]), x[:, 128:]], axis=1)
                mean = jnp.sum(x, axis=1, keepdims=True) * (1.0 / D)
                stat_buf[0, rows, :] = jnp.broadcast_to(mean, (16, 128))
                c = x - mean
                sq = jnp.where(lane16 == t, jnp.sum(c * c, axis=1, keepdims=True), sq)
                dot = jnp.where(lane16 == t, jnp.sum(c * wrow, axis=1, keepdims=True), dot)
                if never16 is not None and t % 2 == 0:
                    last = sq
                yield
            inv = 1.0 / _round_bf16(jnp.sqrt(_round_bf16(_round_bf16(sq * (1.0 / D)) + EPS)))
            mine = (lane16 >= slabs[0]) & (lane16 <= slabs[-1])
            score = _round_bf16(dot * inv)
            scores[0] = jnp.where(mine & (score == score), score, scores[0])
            for t in slabs:
                stat_buf[1, pl.ds(16 * t, 16), :] = jnp.broadcast_to(inv[:, t:t + 1], (16, 128))

    def normalized(rows, cols=slice(None), factor=None):
        x = x_buf[rows, cols].astype(F32)
        reps = x.shape[1] // 128
        mean = jnp.concatenate([stat_buf[0, rows, :]] * reps, axis=1)
        inv = stat_buf[1, rows, :] if factor is None else stat_buf[1, rows, :] * factor
        inv = jnp.concatenate([inv] * reps, axis=1)
        return x, (x - mean) * inv

    def token_sums(j, which=range(7)):
        for r in range(0, SUB, 16):
            a = normalized(pl.ds(j * STEP + r, 16))[1]
            b = normalized(pl.ds(j * STEP + SUB + r, 16))[1] if 0 in which else a
            for n, v in enumerate(_rhs_sums(a[:, :HD], b[:, :HD], a[:, HD:], b[:, HD:])):
                if n in which:
                    xs_buf.at[j, n][pl.ds(r // 2, 8), :] = _pack(v)

    def project(m, j, n):
        return _dot_nt(_unpack(w_sum[m, n]), _unpack(xs_buf[j, n]))

    def project_q(j, between):
        def emit(rh, ch, v):
            pq_buf[j, ch, pl.ds(rh * HD, HD), :] = v
        _strassen(lambda n: project(0, j, n), emit, between)

    def after(token, v):
        top = jnp.where(never, token, v[:8, :128])
        if v.shape[1] > 128:
            top = jnp.concatenate([top, v[:8, 128:]], axis=1)
        return jnp.concatenate([top, v[8:]], axis=0)

    start_in_order(
        [wr_copy, x_copy(0), wphi_copy, q_copy(1, 1), x_copy(1), q_copy(1, 0), x_copy(2),
         q_copy(0, 0), x_copy(3), q_copy(0, 1), x_copy(4), x_copy(5), w_copy(2), w_copy(1),
         x_copy(6)], 0)
    start_in_order([c for i in range(NB) for c in ffn_copies(i) + wo_copies(i)], 1)
    kv_acc[...] = jnp.zeros(kv_acc.shape, F32)
    z_acc[...] = jnp.zeros(z_acc.shape, F32)
    y_acc[...] = jnp.zeros(y_acc.shape, F32)
    wo_sum[0, pl.ds(0, 8), pl.ds(0, 128)] = jnp.zeros((8, 128), U32)
    wr_copy.wait()
    x_copy(0).wait()
    _advance(token_stats(0, (0,), None))
    never = stat_buf[1, pl.ds(0, 8), :] < 0.0
    never16 = jnp.concatenate([never, never], axis=0)
    zero = never.astype(jnp.int32)[0, 0]
    token_sums(0, (1, 3))
    wphi_copy.wait()
    for g in range(NG):
        fold_buf.at[g][...] = _pack(jnp.concatenate([fold_matrix(g), fold_matrix(g + NG)], axis=1))

    def q_quadrant(rh, kh):
        q_copy(rh, kh).wait()
        return jnp.concatenate([
            _dot_nt(_unpack(fold_buf[g, :, pl.ds(128 * rh, 128)]),
                    w_raw[0, pl.ds(kh * HD, HD), pl.ds(rh * HD + 128 * g, 128)])
            for g in range(NG)], axis=0)

    def first_product(n, lhs):
        lhs = _pack(lhs)
        w_sum.at[0, n][...] = lhs
        return _dot_nt(_unpack(lhs), _unpack(xs_buf[0, n]))

    a22 = q_quadrant(1, 1)
    m4 = first_product(3, a22)
    x_copy(1).wait()
    a21 = q_quadrant(1, 0)
    _advance(token_stats(0, (1,), None))
    token_sums(0, (0, 2, 4, 5, 6))
    m2 = first_product(1, a21 + a22)
    pq_buf[0, 0, pl.ds(HD, HD), :] = m2 + m4
    x_copy(2).wait()
    a11 = q_quadrant(0, 0)
    _advance(token_stats(1, (0,), never16))
    token_sums(1, (1, 3))
    m3 = first_product(2, a11)
    m1 = first_product(0, a11 + a22)
    pq_buf[0, 1, pl.ds(HD, HD), :] = m3 - m2 + m1 + first_product(5, a21 - a11)
    x_copy(3).wait()
    a12 = q_quadrant(0, 1)
    _advance(token_stats(1, (1,), never16))
    m5 = first_product(4, a11 + a12)
    pq_buf[0, 1, pl.ds(0, HD), :] = m3 + m5
    pq_buf[0, 0, pl.ds(0, HD), :] = m4 + m1 - m5 + first_product(6, a12 - a22)
    token_sums(1, (0, 2, 4, 5, 6))

    later = _Deferred()
    for j in range(1, NSTEP - 1):
        if j == 1:
            x_copy(4).wait()
        if j == 3:
            x_copy(5).wait()
            w_copy(2).wait()
        if j == 5:
            w_copy(1).wait()
            x_copy(6).wait()
        stats = token_stats(j + 1, (0, 1), never16)

        def alongside(n, j=j, stats=stats):
            later.tick()
            _advance(stats, (4, 4, 4, 5, 0, 0, 0)[n])
            g, offset = divmod(7 * ((j - 3) % 2) + n, 3)
            if j >= 3 and offset == 0 and g < NG:
                m = 2 if j < 5 else 1
                later.add(2, prepare_weights(m, g, m))
        project_q(j, alongside)
        _advance(stats)
        token_sums(j + 1)
        if j % 2 == 0:
            later.flush()

    top = jnp.max(jnp.max(scores[0], axis=0, keepdims=True), axis=1, keepdims=True)
    token = (16 * lane16 + lax.broadcasted_iota(jnp.int32, (16, 128), 0)).astype(F32)
    cand = jnp.where(scores[0] == top, token, float(S))
    idx = jnp.min(jnp.min(cand, axis=0, keepdims=True), axis=1, keepdims=True)
    idx = jnp.clip(idx.astype(jnp.int32)[0, 0], 0, S - 1)
    slab = pl.ds(pl.multiple_of((idx // 16) * 16, 16), 16)
    pick = lax.broadcasted_iota(jnp.int32, (16, D), 0) == idx % 16
    x_sel = jnp.sum(jnp.where(pick, _round_bf16(normalized(slab)[1]), 0.0), axis=0, keepdims=True)
    for c in range(0, D, 128):
        xb_buf[pl.ds(c, 128), :] = jnp.broadcast_to(x_sel[:, c:c + 128], (128, 128)).T

    def matvec(acc, rows, load, column, last):
        acc = list(acc)
        for r0 in range(0, rows, 32):
            slabs = [(load(r).astype(F32), column(r)) for r in range(r0, r0 + 32, 8)]
            for e in range(2):
                if last is not None:
                    acc[e] = jnp.where(never, last, acc[e])
                for w, col in slabs:
                    acc[e] = acc[e] + w[:, 128 * e:128 * e + 128] * col
                last = acc[e]
        return acc, last

    def ffn(i):
        last = None
        act = []
        for c in range(0, 2 * FC, 256):
            acc, last = matvec([jnp.zeros((8, 128), F32)] * 2, D,
                               lambda r: wgu_buf[i, pl.ds(r, 8), pl.ds(c, 256)],
                               lambda r: xb_buf[pl.ds(r, 8), :], last)
            act += [_round_bf16(jnp.sum(a, axis=0, keepdims=True)) for a in acc]
        act = jnp.concatenate(act, axis=1)
        h = _round_bf16(_round_bf16(_silu_of_twice(0.5 * act[:, :FC])) * act[:, FC:])
        ys = [[y_acc[:, pl.ds(n + e, 128)] for e in (0, 128)] for n in range(0, D, 256)]
        for c in range(0, FC, 128):
            hb = jnp.broadcast_to(h[:, c:c + 128], (128, 128)).T
            for n in range(D // 256):
                ys[n], last = matvec(ys[n], 128,
                                     lambda r: wd_buf[i, pl.ds(c + r, 8), pl.ds(256 * n, 256)],
                                     lambda r: hb[r:r + 8], last)
        y_acc[...] = jnp.concatenate([y for pair in ys for y in pair], axis=1)

    def phase_b(i, carry):
        for c in ffn_copies(i):
            c.wait()

        @pl.when(i > 0)
        def _():
            for c in wo_copies(i - 1):
                c.wait()

        for t in range(2):
            def emit_k(rh, ch, v, t=t):
                for p in range(NPAIR // 2):
                    pair = rh * (NPAIR // 2) + p
                    pos, pos_sum, neg, neg_sum = _dual_exp(v[64 * p:64 * p + 64])
                    pos_scale = pltpu.reciprocal(pos_sum, approx=True)
                    neg_scale = pltpu.reciprocal(neg_sum, approx=True)
                    phi = [e * pos_scale for e in pos] + [e * neg_scale for e in neg]
                    z_acc[pair] += jnp.concatenate(phi, axis=0)
                    phik_buf.at[pair, 2 * t + ch][...] = _pack(jnp.concatenate(
                        [jnp.concatenate(phi[:8], axis=0), jnp.concatenate(phi[8:], axis=0)],
                        axis=1))
            _strassen(lambda n: project(1, 2 * i + t, n), emit_k)

        prepare_weights(3, (i + NB - 1) % NB, jnp.where(i > 0, 3, 0))()
        ffn(i)

        for t in range(2):
            def emit_v(rh, ch, v, t=t):
                for p in range(0, NPAIR // 2, 2):
                    vt_buf.at[(rh * (NPAIR // 2) + p) // 2, 2 * t + ch][...] = _pack(jnp.concatenate(
                        [v[64 * p:64 * p + 64], v[64 * p + 64:64 * p + 128]], axis=1))

            def product(n, t=t):
                rhs = xs_buf[2 * i + t, n]
                if (t, n) == (0, 2):
                    rhs = after(wo_sum[0, pl.ds(0, 8), pl.ds(0, 128)], rhs)
                return _dot_nt(_unpack(w_sum[2, n]), _unpack(rhs))
            _strassen(product, emit_v)
            for p in range(NPAIR):
                vt = jnp.concatenate(
                    [vt_buf[p // 2, u, :, pl.ds(128 * (p % 2), 128)] for u in (2 * t, 2 * t + 1)],
                    axis=1)
                phi = jnp.concatenate([jnp.concatenate(
                    [phik_buf[p, u, :, pl.ds(128 * e, 128)] for e in range(2)], axis=0)
                    for u in (2 * t, 2 * t + 1)], axis=1)
                kv_acc[p] += _dot_nt(_unpack(vt), _unpack(phi))
        return carry

    lax.fori_loop(0, NB, phase_b, 0)

    for c in wo_copies(NB - 1):
        c.wait()
    prepare_weights(3, NB - 1, 3)()
    y = _round_bf16(jnp.sum(y_acc[...], axis=0, keepdims=True))
    y = _round_bf16(y * _round_bf16(0.5 + 0.5 * jnp.tanh(0.5 * top)))
    upd_buf[0] = jnp.zeros((8, D), F32)
    upd_buf[1] = jnp.where(lax.broadcasted_iota(jnp.int32, (8, D), 0) == idx % 8, 0.5 * y, 0.0)

    own = (lax.broadcasted_iota(jnp.int32, (64, 128), 0) // DH
           == lax.broadcasted_iota(jnp.int32, (64, 128), 1) % 2)
    for p in range(NPAIR // 2):
        kvb_buf.at[p][...] = _pack(jnp.concatenate(
            [jnp.where(own, kv_acc[p + NPAIR // 2 * u], 0.0) for u in range(2)], axis=1))
    for p in range(NPAIR):
        z_acc[p] = jnp.broadcast_to(jnp.sum(z_acc[p], axis=1, keepdims=True), (128, 128))

    later = _Deferred()
    due = []

    def attend_pairs(j, p):
        odd = lax.broadcasted_iota(jnp.int32, (8, SUB), 0) % 2 == 1
        o = []
        for u in range(2):
            pair = p + NPAIR // 2 * u
            for ch in range(2):
                pos, pos_sum, neg, neg_sum = _dual_exp(pq_buf[j, ch, pl.ds(64 * pair, 64), :])
                ratio = pos_sum * pltpu.reciprocal(neg_sum, approx=True)
                phi = pos + [e * ratio for e in neg]
                den = _tree([phi[t] * z_acc[pair, pl.ds(8 * t, 8), :] for t in range(16)], jnp.add)
                scale = pltpu.reciprocal(_allreduce(den, jnp.add) + 1e-6 * pos_sum, approx=True)
                other = pltpu.roll(scale, 1, 0)
                scale = jnp.concatenate(
                    [jnp.where(odd, other, scale)] * 4 + [jnp.where(odd, scale, other)] * 4, axis=0)
                num = _dot(_unpack(kvb_buf[p, :, pl.ds(128 * u, 128)]),
                           jnp.concatenate(phi, axis=0).astype(BF16))
                o.append(num * scale)

        def store():
            os_buf.at[j % 2][pl.ds(32 * p, 32), :] = _pack(jnp.concatenate(_rhs_sums(*o), axis=1))
        later.add(1, store)

    def attend(j):
        def between(n):
            if n >= 0:
                later.tick()
            if j < NSTEP:
                for p in ((0,), (1, 2), (3,), (4,), (5,), (6,), (7,), ())[n + 1]:
                    attend_pairs(j, p)
        between(-1)
        return between

    def finish(j, rh, ch, v):
        cols = pl.ds(rh * HD, HD)
        s = v.T
        for r in range(0, SUB, 16):
            row0 = j * STEP + ch * SUB + r
            x, half_xn = normalized(pl.ds(row0, 16), cols, 0.5)
            half_upd = jnp.concatenate([
                upd_buf[(idx // 8 == row0 // 8 + e).astype(jnp.int32), :, cols]
                for e in range(2)], axis=0)
            gate = _silu_of_twice(half_xn + half_upd)
            out_buf[pl.ds(row0, 16), cols] = (x + s[r:r + 16] * gate).astype(BF16)
        if j == NSTEP - 1:
            last_out_copy(rh, ch).start()
        elif (rh, ch) == (1, 1):
            out_copy(j).start()
        seen = out_buf[pl.ds(pl.multiple_of(zero * 16, 16), 16),
                       pl.ds(pl.multiple_of(zero * 128 + HD, 128), 128)]
        later.add(3, lambda: due.append(pltpu.bitcast(seen, U32)))

    project_q(NSTEP - 1, attend(0))
    for j in range(NSTEP):
        def emit(rh, ch, v, j=j):
            if j == NSTEP - 1:
                finish(j, rh, ch, v)
            else:
                later.add(1, lambda: finish(j, rh, ch, v))

        def product(n, j=j):
            rhs = os_buf[j % 2, :, pl.ds(SUB * n, SUB)]
            while due:
                rhs = after(due.pop(), rhs)
            return _dot(_unpack(wo_sum[n]), _unpack(rhs))
        _strassen(product, emit, attend(j + 1))
    for j in range(NSTEP - 1):
        out_copy(j).wait()
    for rh in range(2):
        for ch in range(2):
            last_out_copy(rh, ch).wait()


@jax.jit
def pallas_recurrent_scan__linear_kernel_hedgehog__moe_arch_mod__prompt_kernel(
    A_x: jax.Array,
    A_wqkv: jax.Array,
    A_w_phi: jax.Array,
    A_wo: jax.Array,
    B_x: jax.Array,
    B_w_r: jax.Array,
    B_w_gate: jax.Array,
    B_w_up: jax.Array,
    B_w_down: jax.Array,
):
    del B_x
    scratch = [
        pltpu.VMEM((S, D), BF16),
        pltpu.VMEM((NSTEP, 7, SUB // 2, HD), U32),
        pltpu.VMEM((2, S, 128), F32),
        pltpu.VMEM((4, D, D), BF16),
        pltpu.VMEM((3, 7, HD // 2, HD), U32),
        pltpu.VMEM((7, HD // 2, HD), U32),
        pltpu.VMEM((H * DH, DH), BF16),
        pltpu.VMEM((NG, 64, 256), U32),
        pltpu.VMEM((8, 128), BF16),
        pltpu.VMEM((NSTEP, 2, D, SUB), F32),
        pltpu.VMEM((NPAIR // 2, 4, 32, 256), U32),
        pltpu.VMEM((NPAIR, 4, 32, 256), U32),
        pltpu.VMEM((NPAIR, 64, 128), F32),
        pltpu.VMEM((NPAIR, 128, 128), F32),
        pltpu.VMEM((NPAIR // 2, 32, 256), U32),
        pltpu.VMEM((2, HD // 2, 7 * SUB), U32),
        pltpu.VMEM((NB, D, 2 * FC), BF16),
        pltpu.VMEM((NB, FC, D), BF16),
        pltpu.VMEM((D, 128), F32),
        pltpu.VMEM((8, D), F32),
        pltpu.VMEM((2, 8, D), F32),
        pltpu.VMEM((S, D), BF16),
        pltpu.SemaphoreType.DMA((len(X_CUTS) - 1,)),
        pltpu.SemaphoreType.DMA((4,)),
        pltpu.SemaphoreType.DMA((2,)),
        pltpu.SemaphoreType.DMA((2,)),
        pltpu.SemaphoreType.DMA((5 * NB,)),
        pltpu.SemaphoreType.DMA((NSTEP - 1,)),
        pltpu.SemaphoreType.DMA((4,)),
        pltpu.SemaphoreType.REGULAR,
    ]
    any_spec = pl.BlockSpec(memory_space=pl.ANY)
    out = pl.pallas_call(
        _kernel,
        out_shape=jax.ShapeDtypeStruct((S, D), BF16),
        in_specs=[any_spec] * 8,
        out_specs=any_spec,
        scratch_shapes=scratch,
        compiler_params=pltpu.CompilerParams(vmem_limit_bytes=120 * 2**20,
                                             disable_semaphore_checks=True),
        name="hedgehog_mod",
    )(
        A_x.reshape(S, D),
        A_wqkv,
        A_w_phi.reshape(H * DH, DH),
        A_wo,
        B_w_r.reshape(8, 128),
        B_w_gate,
        B_w_up,
        B_w_down,
    )
    return out.reshape(1, S, D)
```

```python
import math

import jax
import jax.numpy as jnp
from jax import lax
import jax.experimental.pallas as pl
import jax.experimental.pallas.tpu as pltpu

S, D, H, DH, F = 2048, 1024, 32, 32, 3584
SUB = 128
STEP = 2 * SUB
NSTEP = S // STEP
NB = 4
FC = F // NB
HD = D // 2
NG = HD // 128
NPAIR = H // 2
X_CUTS = (0, 1, 2, 3, 4, 8, 12, 16)
LOG2E = math.log2(math.e)
EPS = 1.0013580322265625e-05
F32, BF16, U32 = jnp.float32, jnp.bfloat16, jnp.uint32


def _dot(a, b):
    return jnp.dot(a, b, preferred_element_type=F32)


def _dot_nt(a, b):
    return lax.dot_general(a, b, (((1,), (1,)), ((), ())), preferred_element_type=F32)


def _round_bf16(v):
    return v.astype(BF16).astype(F32)


def _pack(v):
    return pltpu.bitcast(v.astype(BF16), U32)


def _unpack(v):
    return pltpu.bitcast(v, BF16)


def _aligned(i, n):
    return i if isinstance(i, int) else pl.multiple_of(i, n)


def _silu_of_twice(h):
    return h + h * jnp.tanh(h)


def _allreduce(v, op):
    v = op(v, pltpu.roll(v, 4, 0))
    return op(v, pltpu.roll(v, 2, 0))


def _tree(vals, op):
    while len(vals) > 1:
        vals = [op(a, b) for a, b in zip(vals[::2], vals[1::2])]
    return vals[0]


def _dual_exp(p):
    ps = [p[8 * j:8 * j + 8] for j in range(8)]
    hi = _allreduce(_tree(ps, jnp.maximum), jnp.maximum)
    lo = _allreduce(_tree(ps, jnp.minimum), jnp.minimum)
    pos = [jnp.exp2(v - hi) for v in ps]
    neg = [jnp.exp2(lo - v) for v in ps]
    return (pos, _allreduce(_tree(pos, jnp.add), jnp.add),
            neg, _allreduce(_tree(neg, jnp.add), jnp.add))


def _lhs_sums(a11, a12, a21, a22):
    return (a11 + a22, a21 + a22, a11, a22, a11 + a12, a21 - a11, a12 - a22)


def _rhs_sums(b11, b12, b21, b22):
    return (b11 + b22, b11, b12 - b22, b21 - b11, b22, b11 + b12, b21 + b22)


def _strassen(prod, emit, between=lambda n: None):
    m2 = prod(1)
    between(0)
    m4 = prod(3)
    emit(1, 0, m2 + m4)
    between(1)
    m3 = prod(2)
    c22 = m3 - m2
    between(2)
    m5 = prod(4)
    emit(0, 1, m3 + m5)
    c11 = m4 - m5
    between(3)
    m1 = prod(0)
    c11 = c11 + m1
    c22 = c22 + m1
    between(4)
    emit(0, 0, c11 + prod(6))
    between(5)
    emit(1, 1, c22 + prod(5))
    between(6)


class _Deferred:
    def __init__(self):
        self.now = 0
        self.items = []

    def add(self, delay, fn):
        self.items.append((self.now + delay, fn))

    def tick(self):
        self.now += 1
        due = [fn for t, fn in self.items if t <= self.now]
        self.items = [(t, fn) for t, fn in self.items if t > self.now]
        for fn in due:
            fn()

    def flush(self):
        items, self.items = self.items, []
        for _, fn in items:
            fn()


def _advance(steps, count=STEP):
    for _ in range(count):
        next(steps, None)


def _kernel(x_hbm, wqkv_hbm, wphi_hbm, wo_hbm, wr_hbm, wg_hbm, wu_hbm, wd_hbm,
            out_hbm,
            x_buf, xs_buf, stat_buf, w_raw, w_sum, wo_sum, wphi_buf, fold_buf, wr_buf,
            pq_buf, vt_buf, phik_buf, kv_acc, z_acc, kvb_buf, os_buf,
            wgu_buf, wd_buf, xb_buf, y_acc, upd_buf, out_buf,
            sem_x, sem_q, sem_w, sem_s, sem_f, sem_o, sem_last, sem_order):
    def x_copy(n):
        rows = pl.ds(X_CUTS[n] * SUB, (X_CUTS[n + 1] - X_CUTS[n]) * SUB)
        return pltpu.make_async_copy(x_hbm.at[rows], x_buf.at[rows], sem_x.at[n])

    def q_copy(rh, kh):
        blk = (pl.ds(kh * HD, HD), pl.ds(rh * HD, HD))
        return pltpu.make_async_copy(wqkv_hbm.at[blk], w_raw.at[0].at[blk], sem_q.at[2 * rh + kh])

    def w_copy(m):
        return pltpu.make_async_copy(wqkv_hbm.at[:, pl.ds(m * D, D)], w_raw.at[m], sem_w.at[m - 1])

    def ffn_copies(i):
        cols = pl.ds(i * FC, FC)
        return (
            pltpu.make_async_copy(wg_hbm.at[:, cols], wgu_buf.at[i, :, pl.ds(0, FC)], sem_f.at[i]),
            pltpu.make_async_copy(wu_hbm.at[:, cols], wgu_buf.at[i, :, pl.ds(FC, FC)],
                                  sem_f.at[NB + i]),
            pltpu.make_async_copy(wd_hbm.at[cols], wd_buf.at[i], sem_f.at[2 * NB + i]),
        )

    def wo_copies(g):
        return tuple(
            pltpu.make_async_copy(wo_hbm.at[:, cols], w_raw.at[3, :, cols],
                                  sem_f.at[(3 + half) * NB + g])
            for half in range(2)
            for cols in [pl.ds(_aligned(128 * (g + NG * half), 128), 128)])

    def out_copy(j):
        rows = pl.ds(j * STEP, STEP)
        return pltpu.make_async_copy(out_buf.at[rows], out_hbm.at[rows], sem_o.at[j])

    def last_out_copy(rh, ch):
        blk = (pl.ds(S - STEP + ch * SUB, SUB), pl.ds(rh * HD, HD))
        return pltpu.make_async_copy(out_buf.at[blk], out_hbm.at[blk], sem_last.at[2 * rh + ch])

    wphi_copy = pltpu.make_async_copy(wphi_hbm, wphi_buf, sem_s.at[0])
    wr_copy = pltpu.make_async_copy(wr_hbm, wr_buf, sem_s.at[1])

    def start_in_order(copies, priority):
        for c in copies:
            c.start(priority=priority)
            pl.semaphore_signal(sem_order, 1)
            pl.semaphore_wait(sem_order, 1)

    def fold_matrix(g):
        r = lax.broadcasted_iota(jnp.int32, (128, DH), 0)
        f = lax.broadcasted_iota(jnp.int32, (128, DH), 1)
        sel = jnp.where((r % 64) // 2 == f, 1.0, 0.0).astype(BF16)
        t = _dot_nt(sel, wphi_buf[pl.ds(128 * g, 128), :])
        r = lax.broadcasted_iota(jnp.int32, (128, 128), 0)
        c = lax.broadcasted_iota(jnp.int32, (128, 128), 1)
        return jnp.where(2 * (r // 64) + r % 2 == c // DH, t * LOG2E, 0.0)

    def prepare_weights(m, g, src):
        def block(half, k0):
            w = w_raw[src, pl.ds(k0, 256), pl.ds(_aligned(128 * (g + NG * half), 128), 128)]
            if m == 1:
                return _dot_nt(_unpack(fold_buf[g, :, pl.ds(128 * half, 128)]), w)
            return w.T.astype(F32)

        blocks = {k0: (block(0, k0), block(0, HD + k0), block(1, k0), block(1, HD + k0))
                  for k0 in range(0, HD, 256)}

        def store():
            dst = wo_sum if m == 3 else w_sum.at[m]
            for k0, quad in blocks.items():
                for n, v in enumerate(_lhs_sums(*quad)):
                    dst.at[n][pl.ds(_aligned(64 * g, 64), 64), pl.ds(k0, 256)] = _pack(v)
        return store

    lane16 = lax.broadcasted_iota(jnp.int32, (16, 128), 1)
    scores = [jnp.full((16, 128), -jnp.inf, F32)]

    def token_stats(j, halves):
        wr = wr_buf[...].astype(F32)
        wrow = jnp.concatenate(
            [jnp.broadcast_to(wr[c:c + 1], (16, 128)) for c in range(8)], axis=1)
        for half in halves:
            slabs = range((2 * j + half) * SUB // 16, (2 * j + half + 1) * SUB // 16)
            sq = dot = jnp.zeros((16, 128), F32)
            for t in slabs:
                rows = pl.ds(16 * t, 16)
                x = x_buf[rows, :].astype(F32)
                mean = jnp.sum(x, axis=1, keepdims=True) * (1.0 / D)
                stat_buf[0, rows, :] = jnp.broadcast_to(mean, (16, 128))
                c = x - mean
                sq = jnp.where(lane16 == t, jnp.sum(c * c, axis=1, keepdims=True), sq)
                dot = jnp.where(lane16 == t, jnp.sum(c * wrow, axis=1, keepdims=True), dot)
                yield
            inv = 1.0 / _round_bf16(jnp.sqrt(_round_bf16(_round_bf16(sq * (1.0 / D)) + EPS)))
            mine = (lane16 >= slabs[0]) & (lane16 <= slabs[-1])
            score = _round_bf16(dot * inv)
            scores[0] = jnp.where(mine & (score == score), score, scores[0])
            for t in slabs:
                stat_buf[1, pl.ds(16 * t, 16), :] = jnp.broadcast_to(inv[:, t:t + 1], (16, 128))

    def normalized(rows, cols=slice(None), factor=None):
        x = x_buf[rows, cols].astype(F32)
        reps = x.shape[1] // 128
        mean = jnp.concatenate([stat_buf[0, rows, :]] * reps, axis=1)
        inv = stat_buf[1, rows, :] if factor is None else stat_buf[1, rows, :] * factor
        inv = jnp.concatenate([inv] * reps, axis=1)
        return x, (x - mean) * inv

    def token_sums(j, which=range(7)):
        for r in range(0, SUB, 16):
            a = normalized(pl.ds(j * STEP + r, 16))[1]
            b = normalized(pl.ds(j * STEP + SUB + r, 16))[1] if 0 in which else a
            for n, v in enumerate(_rhs_sums(a[:, :HD], b[:, :HD], a[:, HD:], b[:, HD:])):
                if n in which:
                    xs_buf.at[j, n][pl.ds(r // 2, 8), :] = _pack(v)

    def project(m, j, n):
        return _dot_nt(_unpack(w_sum[m, n]), _unpack(xs_buf[j, n]))

    def project_q(j, between):
        def emit(rh, ch, v):
            pq_buf[j, ch, pl.ds(rh * HD, HD), :] = v
        _strassen(lambda n: project(0, j, n), emit, between)

    def after(token, v):
        top = jnp.where(never, token, v[:8, :128])
        if v.shape[1] > 128:
            top = jnp.concatenate([top, v[:8, 128:]], axis=1)
        return jnp.concatenate([top, v[8:]], axis=0)

    start_in_order(
        [wr_copy, x_copy(0), wphi_copy, q_copy(1, 1), x_copy(1), q_copy(1, 0), x_copy(2),
         q_copy(0, 0), x_copy(3), q_copy(0, 1), x_copy(4), x_copy(5), w_copy(2), w_copy(1),
         x_copy(6)], 0)
    start_in_order([c for i in range(NB) for c in ffn_copies(i) + wo_copies(i)], 1)
    kv_acc[...] = jnp.zeros(kv_acc.shape, F32)
    z_acc[...] = jnp.zeros(z_acc.shape, F32)
    y_acc[...] = jnp.zeros(y_acc.shape, F32)
    wo_sum[0, pl.ds(0, 8), pl.ds(0, 128)] = jnp.zeros((8, 128), U32)
    wr_copy.wait()
    x_copy(0).wait()
    _advance(token_stats(0, (0,)))
    never = stat_buf[1, pl.ds(0, 8), :] < 0.0
    zero = never.astype(jnp.int32)[0, 0]
    token_sums(0, (1, 3))
    wphi_copy.wait()
    for g in range(NG):
        fold_buf.at[g][...] = _pack(jnp.concatenate([fold_matrix(g), fold_matrix(g + NG)], axis=1))

    def q_quadrant(rh, kh):
        q_copy(rh, kh).wait()
        return jnp.concatenate([
            _dot_nt(_unpack(fold_buf[g, :, pl.ds(128 * rh, 128)]),
                    w_raw[0, pl.ds(kh * HD, HD), pl.ds(rh * HD + 128 * g, 128)])
            for g in range(NG)], axis=0)

    def first_product(n, lhs):
        lhs = _pack(lhs)
        w_sum.at[0, n][...] = lhs
        return _dot_nt(_unpack(lhs), _unpack(xs_buf[0, n]))

    a22 = q_quadrant(1, 1)
    m4 = first_product(3, a22)
    x_copy(1).wait()
    a21 = q_quadrant(1, 0)
    _advance(token_stats(0, (1,)))
    token_sums(0, (0, 2, 4, 5, 6))
    m2 = first_product(1, a21 + a22)
    pq_buf[0, 0, pl.ds(HD, HD), :] = m2 + m4
    x_copy(2).wait()
    a11 = q_quadrant(0, 0)
    _advance(token_stats(1, (0,)))
    token_sums(1, (1, 3))
    m3 = first_product(2, a11)
    m1 = first_product(0, a11 + a22)
    pq_buf[0, 1, pl.ds(HD, HD), :] = m3 - m2 + m1 + first_product(5, a21 - a11)
    x_copy(3).wait()
    a12 = q_quadrant(0, 1)
    _advance(token_stats(1, (1,)))
    m5 = first_product(4, a11 + a12)
    pq_buf[0, 1, pl.ds(0, HD), :] = m3 + m5
    pq_buf[0, 0, pl.ds(0, HD), :] = m4 + m1 - m5 + first_product(6, a12 - a22)
    token_sums(1, (0, 2, 4, 5, 6))

    later = _Deferred()
    for j in range(1, NSTEP - 1):
        if j == 1:
            x_copy(4).wait()
        if j == 3:
            x_copy(5).wait()
            w_copy(2).wait()
        if j == 5:
            w_copy(1).wait()
            x_copy(6).wait()
        stats = token_stats(j + 1, (0, 1))

        def alongside(n, j=j, stats=stats):
            later.tick()
            _advance(stats, (4, 4, 4, 5, 0, 0, 0)[n])
            g, offset = divmod(7 * ((j - 3) % 2) + n, 3)
            if j >= 3 and offset == 0 and g < NG:
                m = 2 if j < 5 else 1
                later.add(2, prepare_weights(m, g, m))
        project_q(j, alongside)
        _advance(stats)
        token_sums(j + 1)
        if j % 2 == 0:
            later.flush()

    top = jnp.max(jnp.max(scores[0], axis=0, keepdims=True), axis=1, keepdims=True)
    token = (16 * lane16 + lax.broadcasted_iota(jnp.int32, (16, 128), 0)).astype(F32)
    cand = jnp.where(scores[0] == top, token, float(S))
    idx = jnp.min(jnp.min(cand, axis=0, keepdims=True), axis=1, keepdims=True)
    idx = jnp.clip(idx.astype(jnp.int32)[0, 0], 0, S - 1)
    slab = pl.ds(pl.multiple_of((idx // 16) * 16, 16), 16)
    pick = lax.broadcasted_iota(jnp.int32, (16, D), 0) == idx % 16
    x_sel = jnp.sum(jnp.where(pick, _round_bf16(normalized(slab)[1]), 0.0), axis=0, keepdims=True)
    for c in range(0, D, 128):
        xb_buf[pl.ds(c, 128), :] = jnp.broadcast_to(x_sel[:, c:c + 128], (128, 128)).T

    def matvec(acc, rows, load, column, last):
        acc = list(acc)
        for r0 in range(0, rows, 32):
            slabs = [(load(r).astype(F32), column(r)) for r in range(r0, r0 + 32, 8)]
            for e in range(2):
                if last is not None:
                    acc[e] = jnp.where(never, last, acc[e])
                for w, col in slabs:
                    acc[e] = acc[e] + w[:, 128 * e:128 * e + 128] * col
                last = acc[e]
        return acc, last

    def ffn(i):
        last = None
        act = []
        for c in range(0, 2 * FC, 256):
            acc, last = matvec([jnp.zeros((8, 128), F32)] * 2, D,
                               lambda r: wgu_buf[i, pl.ds(r, 8), pl.ds(c, 256)],
                               lambda r: xb_buf[pl.ds(r, 8), :], last)
            act += [_round_bf16(jnp.sum(a, axis=0, keepdims=True)) for a in acc]
        act = jnp.concatenate(act, axis=1)
        h = _round_bf16(_round_bf16(_silu_of_twice(0.5 * act[:, :FC])) * act[:, FC:])
        ys = [[y_acc[:, pl.ds(n + e, 128)] for e in (0, 128)] for n in range(0, D, 256)]
        for c in range(0, FC, 128):
            hb = jnp.broadcast_to(h[:, c:c + 128], (128, 128)).T
            for n in range(D // 256):
                ys[n], last = matvec(ys[n], 128,
                                     lambda r: wd_buf[i, pl.ds(c + r, 8), pl.ds(256 * n, 256)],
                                     lambda r: hb[r:r + 8], last)
        y_acc[...] = jnp.concatenate([y for pair in ys for y in pair], axis=1)

    def phase_b(i, carry):
        for c in ffn_copies(i):
            c.wait()

        @pl.when(i > 0)
        def _():
            for c in wo_copies(i - 1):
                c.wait()

        for t in range(2):
            def emit_k(rh, ch, v, t=t):
                for p in range(NPAIR // 2):
                    pair = rh * (NPAIR // 2) + p
                    pos, pos_sum, neg, neg_sum = _dual_exp(v[64 * p:64 * p + 64])
                    pos_scale = pltpu.reciprocal(pos_sum, approx=True)
                    neg_scale = pltpu.reciprocal(neg_sum, approx=True)
                    phi = [e * pos_scale for e in pos] + [e * neg_scale for e in neg]
                    z_acc[pair] += jnp.concatenate(phi, axis=0)
                    phik_buf.at[pair, 2 * t + ch][...] = _pack(jnp.concatenate(
                        [jnp.concatenate(phi[:8], axis=0), jnp.concatenate(phi[8:], axis=0)],
                        axis=1))
            _strassen(lambda n: project(1, 2 * i + t, n), emit_k)

        prepare_weights(3, (i + NB - 1) % NB, jnp.where(i > 0, 3, 0))()
        ffn(i)

        for t in range(2):
            def emit_v(rh, ch, v, t=t):
                for p in range(0, NPAIR // 2, 2):
                    vt_buf.at[(rh * (NPAIR // 2) + p) // 2, 2 * t + ch][...] = _pack(jnp.concatenate(
                        [v[64 * p:64 * p + 64], v[64 * p + 64:64 * p + 128]], axis=1))

            def product(n, t=t):
                rhs = xs_buf[2 * i + t, n]
                if (t, n) == (0, 2):
                    rhs = after(wo_sum[0, pl.ds(0, 8), pl.ds(0, 128)], rhs)
                return _dot_nt(_unpack(w_sum[2, n]), _unpack(rhs))
            _strassen(product, emit_v)
            for p in range(NPAIR):
                vt = jnp.concatenate(
                    [vt_buf[p // 2, u, :, pl.ds(128 * (p % 2), 128)] for u in (2 * t, 2 * t + 1)],
                    axis=1)
                phi = jnp.concatenate([jnp.concatenate(
                    [phik_buf[p, u, :, pl.ds(128 * e, 128)] for e in range(2)], axis=0)
                    for u in (2 * t, 2 * t + 1)], axis=1)
                kv_acc[p] += _dot_nt(_unpack(vt), _unpack(phi))
        return carry

    lax.fori_loop(0, NB, phase_b, 0)

    for c in wo_copies(NB - 1):
        c.wait()
    prepare_weights(3, NB - 1, 3)()
    y = _round_bf16(jnp.sum(y_acc[...], axis=0, keepdims=True))
    y = _round_bf16(y * _round_bf16(0.5 + 0.5 * jnp.tanh(0.5 * top)))
    upd_buf[0] = jnp.zeros((8, D), F32)
    upd_buf[1] = jnp.where(lax.broadcasted_iota(jnp.int32, (8, D), 0) == idx % 8, 0.5 * y, 0.0)

    own = (lax.broadcasted_iota(jnp.int32, (64, 128), 0) // DH
           == lax.broadcasted_iota(jnp.int32, (64, 128), 1) % 2)
    for p in range(NPAIR // 2):
        kvb_buf.at[p][...] = _pack(jnp.concatenate(
            [jnp.where(own, kv_acc[p + NPAIR // 2 * u], 0.0) for u in range(2)], axis=1))
    for p in range(NPAIR):
        z_acc[p] = jnp.broadcast_to(jnp.sum(z_acc[p], axis=1, keepdims=True), (128, 128))

    later = _Deferred()
    due = []

    def attend_pairs(j, p):
        odd = lax.broadcasted_iota(jnp.int32, (8, SUB), 0) % 2 == 1
        o = []
        for u in range(2):
            pair = p + NPAIR // 2 * u
            for ch in range(2):
                pos, pos_sum, neg, neg_sum = _dual_exp(pq_buf[j, ch, pl.ds(64 * pair, 64), :])
                ratio = pos_sum * pltpu.reciprocal(neg_sum, approx=True)
                phi = pos + [e * ratio for e in neg]
                den = _tree([phi[t] * z_acc[pair, pl.ds(8 * t, 8), :] for t in range(16)], jnp.add)
                scale = pltpu.reciprocal(_allreduce(den, jnp.add) + 1e-6 * pos_sum, approx=True)
                other = pltpu.roll(scale, 1, 0)
                scale = jnp.concatenate(
                    [jnp.where(odd, other, scale)] * 4 + [jnp.where(odd, scale, other)] * 4, axis=0)
                num = _dot(_unpack(kvb_buf[p, :, pl.ds(128 * u, 128)]),
                           jnp.concatenate(phi, axis=0).astype(BF16))
                o.append(num * scale)

        def store():
            os_buf.at[j % 2][pl.ds(32 * p, 32), :] = _pack(jnp.concatenate(_rhs_sums(*o), axis=1))
        later.add(1, store)

    def attend(j):
        def between(n):
            if n >= 0:
                later.tick()
            if j < NSTEP:
                for p in ((0,), (1, 2), (3,), (4,), (5,), (6,), (7,), ())[n + 1]:
                    attend_pairs(j, p)
        between(-1)
        return between

    def finish(j, rh, ch, v):
        cols = pl.ds(rh * HD, HD)
        s = v.T
        for r in range(0, SUB, 16):
            row0 = j * STEP + ch * SUB + r
            x, half_xn = normalized(pl.ds(row0, 16), cols, 0.5)
            half_upd = jnp.concatenate([
                upd_buf[(idx // 8 == row0 // 8 + e).astype(jnp.int32), :, cols]
                for e in range(2)], axis=0)
            gate = _silu_of_twice(half_xn + half_upd)
            out_buf[pl.ds(row0, 16), cols] = (x + s[r:r + 16] * gate).astype(BF16)
        if j == NSTEP - 1:
            last_out_copy(rh, ch).start()
        elif (rh, ch) == (1, 1):
            out_copy(j).start()
        seen = out_buf[pl.ds(pl.multiple_of(zero * 16, 16), 16),
                       pl.ds(pl.multiple_of(zero * 128 + HD, 128), 128)]
        later.add(3, lambda: due.append(pltpu.bitcast(seen, U32)))

    project_q(NSTEP - 1, attend(0))
    for j in range(NSTEP):
        def emit(rh, ch, v, j=j):
            if j == NSTEP - 1:
                finish(j, rh, ch, v)
            else:
                later.add(1, lambda: finish(j, rh, ch, v))

        def product(n, j=j):
            rhs = os_buf[j % 2, :, pl.ds(SUB * n, SUB)]
            while due:
                rhs = after(due.pop(), rhs)
            return _dot(_unpack(wo_sum[n]), _unpack(rhs))
        _strassen(product, emit, attend(j + 1))
    for j in range(NSTEP - 1):
        out_copy(j).wait()
    for rh in range(2):
        for ch in range(2):
            last_out_copy(rh, ch).wait()


@jax.jit
def pallas_recurrent_scan__linear_kernel_hedgehog__moe_arch_mod__prompt_kernel(
    A_x: jax.Array,
    A_wqkv: jax.Array,
    A_w_phi: jax.Array,
    A_wo: jax.Array,
    B_x: jax.Array,
    B_w_r: jax.Array,
    B_w_gate: jax.Array,
    B_w_up: jax.Array,
    B_w_down: jax.Array,
):
    del B_x
    scratch = [
        pltpu.VMEM((S, D), BF16),
        pltpu.VMEM((NSTEP, 7, SUB // 2, HD), U32),
        pltpu.VMEM((2, S, 128), F32),
        pltpu.VMEM((4, D, D), BF16),
        pltpu.VMEM((3, 7, HD // 2, HD), U32),
        pltpu.VMEM((7, HD // 2, HD), U32),
        pltpu.VMEM((H * DH, DH), BF16),
        pltpu.VMEM((NG, 64, 256), U32),
        pltpu.VMEM((8, 128), BF16),
        pltpu.VMEM((NSTEP, 2, D, SUB), F32),
        pltpu.VMEM((NPAIR // 2, 4, 32, 256), U32),
        pltpu.VMEM((NPAIR, 4, 32, 256), U32),
        pltpu.VMEM((NPAIR, 64, 128), F32),
        pltpu.VMEM((NPAIR, 128, 128), F32),
        pltpu.VMEM((NPAIR // 2, 32, 256), U32),
        pltpu.VMEM((2, HD // 2, 7 * SUB), U32),
        pltpu.VMEM((NB, D, 2 * FC), BF16),
        pltpu.VMEM((NB, FC, D), BF16),
        pltpu.VMEM((D, 128), F32),
        pltpu.VMEM((8, D), F32),
        pltpu.VMEM((2, 8, D), F32),
        pltpu.VMEM((S, D), BF16),
        pltpu.SemaphoreType.DMA((len(X_CUTS) - 1,)),
        pltpu.SemaphoreType.DMA((4,)),
        pltpu.SemaphoreType.DMA((2,)),
        pltpu.SemaphoreType.DMA((2,)),
        pltpu.SemaphoreType.DMA((5 * NB,)),
        pltpu.SemaphoreType.DMA((NSTEP - 1,)),
        pltpu.SemaphoreType.DMA((4,)),
        pltpu.SemaphoreType.REGULAR,
    ]
    any_spec = pl.BlockSpec(memory_space=pl.ANY)
    out = pl.pallas_call(
        _kernel,
        out_shape=jax.ShapeDtypeStruct((S, D), BF16),
        in_specs=[any_spec] * 8,
        out_specs=any_spec,
        scratch_shapes=scratch,
        compiler_params=pltpu.CompilerParams(vmem_limit_bytes=120 * 2**20,
                                             disable_semaphore_checks=True),
        name="hedgehog_mod",
    )(
        A_x.reshape(S, D),
        A_wqkv,
        A_w_phi.reshape(H * DH, DH),
        A_wo,
        B_w_r.reshape(8, 128),
        B_w_gate,
        B_w_up,
        B_w_down,
    )
    return out.reshape(1, S, D)
```
